```python
import jax
import jax.numpy as jnp

def _softmax(x, axis=-1):
    return jax.nn.softmax(x, axis=axis)

def _gelu(x):
    return jax.nn.gelu(x, approximate=True)

def _silu(x):
    return jax.nn.silu(x)

def _sigmoid(x):
    return jax.nn.sigmoid(x)

def _layernorm(x, axis=-1, eps=1e-05):
    m = jnp.mean(x, axis=axis, keepdims=True)
    v = jnp.var(x, axis=axis, keepdims=True)
    return (x - m) / jnp.sqrt(v + eps)

def _scatter_add(tgt, idx, src, axis=0):
    return tgt.at[idx].add(src)

def _segment_sum(src, seg, n):
    return jax.ops.segment_sum(src, seg, n)

class _Rng:

    def __init__(self, key):
        self._k = key

    def _next(self):
        self._k, sub = jax.random.split(self._k)
        return sub

    def normal(self, shape):
        return jax.random.normal(self._next(), shape, dtype=jnp.bfloat16)

    def randint(self, lo, hi, shape):
        return jax.random.randint(self._next(), shape, lo, hi, dtype=jnp.int32)

    def uniform(self, shape, lo=0.0, hi=1.0):
        return jax.random.uniform(self._next(), shape, jnp.bfloat16, lo, hi)

    def permutation(self, n):
        return jax.random.permutation(self._next(), n)
kernel_name = 'interleave_layers__memory_aug_recurrent_mem_tr__mixer_s_mlp__prompt'

def setup_inputs():
    _rng = _Rng(jax.random.key(int.from_bytes(__import__("os").urandom(4), "little")))
    _w = lambda a: (lambda t: t.astype(jnp.bfloat16) if jnp.issubdtype(t.dtype, jnp.floating) else t)(jnp.asarray(a))

    def _A_setup():
        B, S, Dm = (1, 2048, 640)
        H, Dh = (32, 192)
        M, seg = (8, 32)
        seg = min(seg, S)
        S = S // seg * seg
        return {'x': _w((lambda *s: _rng.normal(s) * 0.05)(B, S, Dm)), 'mem0': _w((lambda *s: _rng.normal(s) * 0.05)(B, M, Dm)), 'Wq': _w((lambda *s: _rng.normal(s) * 0.05)(Dm, H, Dh) * Dm ** (-0.5)), 'Wk': _w((lambda *s: _rng.normal(s) * 0.05)(Dm, H, Dh) * Dm ** (-0.5)), 'Wv': _w((lambda *s: _rng.normal(s) * 0.05)(Dm, H, Dh) * Dm ** (-0.5)), 'Wo': _w((lambda *s: _rng.normal(s) * 0.05)(H, Dh, Dm) * (H * Dh) ** (-0.5)), 'seg_len': seg}
    _A_in = _A_setup()

    def _B_setup():
        B, S, D, F = (1, 2048, 640, 1536)
        return {'x': _w((lambda *s: _rng.normal(s) * 0.05)(B, S, D)), 'w1': _w((lambda *s: _rng.normal(s) * 0.05)(D, D) * D ** (-0.5)), 'w2': _w((lambda *s: _rng.normal(s) * 0.05)(D, D) * D ** (-0.5)), 'w3': _w((lambda *s: _rng.normal(s) * 0.05)(D, F) * D ** (-0.5)), 'w4': _w((lambda *s: _rng.normal(s) * 0.05)(F, D) * F ** (-0.5))}
    _B_in = _B_setup()
    return {'A_x': _A_in['x'], 'A_mem0': _A_in['mem0'], 'A_Wq': _A_in['Wq'], 'A_Wk': _A_in['Wk'], 'A_Wv': _A_in['Wv'], 'A_Wo': _A_in['Wo'], 'A_seg_len': _A_in['seg_len'], 'B_x': _B_in['x'], 'B_w1': _B_in['w1'], 'B_w2': _B_in['w2'], 'B_w3': _B_in['w3'], 'B_w4': _B_in['w4']}

def reference(A_x, A_mem0, A_Wq, A_Wk, A_Wv, A_Wo, A_seg_len, B_x, B_w1, B_w2, B_w3, B_w4):

    def _A_ref(x, mem0, Wq, Wk, Wv, Wo, seg_len):
        B, S, Dm = x.shape
        H, Dh = (Wq.shape[1], Wq.shape[2])
        M = mem0.shape[1]
        scale = Dh ** (-0.5)
        n_seg = S // seg_len
        L = M + seg_len
        idx = jnp.arange(L)
        mask = (idx[:, None] < M) | (idx[:, None] >= idx[None, :])
        mem = mem0
        outs = []
        for s in range(n_seg):
            xs = x[:, s * seg_len:(s + 1) * seg_len, :].copy()
            h = jnp.concatenate([mem, xs], axis=1)
            q = jnp.einsum('btd,dhe->bhte', h, Wq)
            k = jnp.einsum('btd,dhe->bhte', h, Wk)
            v = jnp.einsum('btd,dhe->bhte', h, Wv)
            scores = jnp.einsum('bhqe,bhke->bhqk', q, k) * scale
            scores = jnp.where(mask[None, None], scores, -1000000000.0)
            p = _softmax(scores, axis=-1)
            o = jnp.einsum('bhqk,bhke->bhqe', p, v)
            o = jnp.einsum('bhte,hed->btd', o, Wo)
            mem = o[:, :M, :].copy()
            outs.append(o[:, M:, :])
        return jnp.concatenate(outs, axis=1)

    def _B_ref(x, w1, w2, w3, w4):
        B, S, D = x.shape
        h = _gelu(_layernorm(x, axis=-1) @ w1)
        c = D // 4
        g0 = jnp.pad(h[:, :, 0 * c:1 * c], ((0, 0), (1, 0), (0, 0)))[:, :S, :]
        g1 = jnp.pad(h[:, :, 1 * c:2 * c], ((0, 0), (0, 1), (0, 0)))[:, 1:, :]
        g2 = jnp.pad(h[:, :, 2 * c:3 * c], ((0, 0), (2, 0), (0, 0)))[:, :S, :]
        g3 = jnp.pad(h[:, :, 3 * c:], ((0, 0), (0, 2), (0, 0)))[:, 2:, :]
        hs = jnp.concatenate([g0, g1, g2, g3], axis=-1) @ w2
        x1 = x + hs
        h2 = _gelu(_layernorm(x1, axis=-1) @ w3) @ w4
        return x1 + h2
    x = A_x
    x = x + _A_ref(_layernorm(x, axis=-1), A_mem0, A_Wq, A_Wk, A_Wv, A_Wo, A_seg_len)
    x = x + _B_ref(_layernorm(x, axis=-1), B_w1, B_w2, B_w3, B_w4)
    x = x + _A_ref(_layernorm(x, axis=-1), A_mem0, A_Wq, A_Wk, A_Wv, A_Wo, A_seg_len)
    x = x + _B_ref(_layernorm(x, axis=-1), B_w1, B_w2, B_w3, B_w4)
    return x
```

```python
import functools

import jax
import jax.numpy as jnp
import numpy as np
from jax import lax
import jax.experimental.pallas as pl
import jax.experimental.pallas.tpu as pltpu

f32 = jnp.float32
bf16 = jnp.bfloat16

S_LEN, D, H, E = 2048, 640, 32, 192
M_MEM, SEG = 8, 32
L = M_MEM + SEG
NSEG = S_LEN // SEG
NP = H // 2
PW = 2 * E
F = 1536
LAG = 3
EPS = 1e-5
NEG = -1e30

NT = (((1,), (1,)), ((), ()))
NN = (((1,), (0,)), ((), ()))


def _dot(a, b, dims):
    return lax.dot_general(a, b, dims, preferred_element_type=f32)


def _ln(x):
    m = jnp.mean(x, axis=-1, keepdims=True)
    xc = x - m
    v = jnp.mean(xc * xc, axis=-1, keepdims=True)
    return xc * lax.rsqrt(v + EPS)


def _gelu(x):
    c = np.float32(np.sqrt(2.0 / np.pi))
    return 0.5 * x * (1.0 + jnp.tanh(c * (x + np.float32(0.044715) * (x * x * x))))


XS_DUMMY = S_LEN
XS_ROWS = S_LEN + SEG
HB_PAD = 8
HB_DUMMY = S_LEN + 2 * HB_PAD + HB_PAD
HB_ROWS = HB_DUMMY + SEG + HB_PAD


def _kernel(x_hbm, mem0_ref, wq_hbm, wk_hbm, wv_hbm, wo_hbm, w1_hbm, w2_hbm, w3_hbm, w4_hbm,
            out_ref,
            x_v, wq, wk, wv, wo, w1, w2, w3, w4, xs, lnx1, lnx2, ybuf, hbuf, mem, sems):
    cps = []
    for i, (src, dst) in enumerate([(x_hbm, x_v), (wq_hbm, wq), (wk_hbm, wk), (wv_hbm, wv), (wo_hbm, wo),
                                    (w1_hbm, w1), (w2_hbm, w2), (w3_hbm, w3), (w4_hbm, w4)]):
        cp = pltpu.make_async_copy(src, dst, sems.at[i])
        cp.start()
        cps.append(cp)

    xs[pl.ds(XS_DUMMY, SEG), :] = jnp.zeros((SEG, D), f32)
    lnx1[pl.ds(XS_DUMMY, SEG), :] = jnp.zeros((SEG, D), f32)
    lnx2[pl.ds(XS_DUMMY, SEG), :] = jnp.zeros((SEG, D), f32)
    ybuf[pl.ds(XS_DUMMY, SEG), :] = jnp.zeros((SEG, D), f32)
    hbuf[pl.ds(0, HB_PAD), :] = jnp.zeros((HB_PAD, D), f32)
    hbuf[pl.ds(HB_PAD + S_LEN, HB_ROWS - HB_PAD - S_LEN), :] = jnp.zeros((HB_ROWS - HB_PAD - S_LEN, D), f32)
    m0 = mem0_ref[...].astype(f32)
    mem[pl.ds(0, M_MEM), :] = m0
    mem[pl.ds(M_MEM, M_MEM), :] = m0

    cps[0].wait()

    def ln_init(s, c):
        r = pl.multiple_of(s * SEG, SEG)
        lnx1[pl.ds(r, SEG), :] = _ln(x_v[pl.ds(r, SEG), :].astype(f32))
        return c
    lax.fori_loop(0, NSEG, ln_init, 0)
    for cp in cps[1:]:
        cp.wait()

    lane128 = lax.broadcasted_iota(jnp.int32, (L, 128), 1)
    lo64 = lane128 < 64
    l80 = lax.broadcasted_iota(jnp.int32, (L, 2 * L), 1)
    row = lax.broadcasted_iota(jnp.int32, (L, 2 * L), 0)
    ha = l80 < L
    key = jnp.where(ha, l80, l80 - L)
    allowed = (row < M_MEM) | (row >= key)
    scale = np.float32(E ** -0.5)
    z40 = jnp.zeros((L, 128), f32)
    lane32 = lax.broadcasted_iota(jnp.int32, (SEG, 128), 1)

    def seg_row(seg, dummy):
        valid = jnp.logical_and(seg >= 0, seg < NSEG)
        return pl.multiple_of(jnp.where(valid, seg * SEG, dummy), 8), valid

    def step(t, carry):
        a_rows = [seg_row(t, XS_DUMMY), seg_row(t - LAG, XS_DUMMY)]
        ba_rows = [seg_row(t - 1, XS_DUMMY), seg_row(t - LAG - 1, XS_DUMMY)]
        bb_rows = [seg_row(t - 2, XS_DUMMY), seg_row(t - LAG - 2, XS_DUMMY)]
        bah_rows = [seg_row(t - 1, HB_DUMMY - HB_PAD)[0] + HB_PAD, seg_row(t - LAG - 1, HB_DUMMY - HB_PAD)[0] + HB_PAD]
        bbh_rows = [seg_row(t - 2, HB_DUMMY - HB_PAD)[0], seg_row(t - LAG - 2, HB_DUMMY - HB_PAD)[0]]
        out_row = pl.multiple_of(jnp.clip(t - LAG - 2, 0, NSEG - 1) * SEG, SEG)
        x0_row = pl.multiple_of(jnp.minimum(t, NSEG - 1) * SEG, SEG)

        st = {}
        h = jnp.concatenate([mem[pl.ds(0, M_MEM), :], lnx1[pl.ds(a_rows[0][0], SEG), :],
                             mem[pl.ds(M_MEM, M_MEM), :], lnx2[pl.ds(a_rows[1][0], SEG), :]], axis=0).astype(bf16)

        def proj(w, p):
            return _dot(h, w[pl.ds(PW * p, PW), :], NT)

        def blk(u):
            t0 = jnp.concatenate([u[:, 0:128], z40], axis=0)
            u1 = u[:, 128:256]
            t1 = jnp.concatenate([jnp.where(lo64, u1, 0.), jnp.where(lo64, 0., u1)], axis=0)
            t2 = jnp.concatenate([z40, u[:, 256:384]], axis=0)
            return jnp.concatenate([t0, t1, t2], axis=1).astype(bf16)

        def a_k(p):
            k = proj(wk, p)
            st['k', p] = [blk(k[L * l:L * l + L]) for l in range(2)]

        def a_q(p):
            q = proj(wq, p)
            st['q', p] = [q[L * l:L * l + L] for l in range(2)]

        def a_v(p):
            v = proj(wv, p)
            st['v', p] = [blk(v[L * l:L * l + L]) for l in range(2)]

        def a_s(p):
            qs, ks = st.pop(('q', p)), st.pop(('k', p))
            ss = [_dot(qs[l], ks[l], NT) for l in range(2)]
            res = []
            for s in ss:
                xm = jnp.where(allowed, s * scale, np.float32(-1e9))
                m0_ = jnp.max(jnp.where(ha, xm, NEG), axis=1, keepdims=True)
                m1_ = jnp.max(jnp.where(ha, NEG, xm), axis=1, keepdims=True)
                pe = jnp.exp(xm - jnp.where(ha, m0_, m1_))
                i0 = 1.0 / jnp.sum(jnp.where(ha, pe, 0.), axis=1, keepdims=True)
                i1 = 1.0 / jnp.sum(jnp.where(ha, 0., pe), axis=1, keepdims=True)
                res.append((pe, i0, i1))
            st['p', p] = res

        def a_pv(p):
            ps, vs = st.pop(('p', p)), st.pop(('v', p))
            outs = []
            for l in range(2):
                pe, i0, i1 = ps[l]
                o = _dot(pe, vs[l], NN)
                outs.append(jnp.concatenate(
                    [o[:, 0:128] * i0, o[:, 128:256] * jnp.where(lo64, i0, i1), o[:, 256:384] * i1], axis=1))
            st['o', p] = jnp.concatenate(outs, axis=0).astype(bf16)

        def a_out(p):
            r = _dot(st.pop(('o', p)), wo[pl.ds(PW * p, PW), :], NN)
            st['acc'] = r if 'acc' not in st else st['acc'] + r

        def a_fin(_):
            acc = st.pop('acc')
            r1, v1 = a_rows[0]
            r2, v2 = a_rows[1]
            mem[pl.ds(0, M_MEM), :] = acc[0:M_MEM]
            xs[pl.ds(r1, SEG), :] = x_v[pl.ds(x0_row, SEG), :].astype(f32) + acc[M_MEM:L]
            mem[pl.ds(M_MEM, M_MEM), :] = jnp.where(v2, acc[L:L + M_MEM], mem[pl.ds(M_MEM, M_MEM), :])
            xs[pl.ds(r2, SEG), :] = xs[pl.ds(r2, SEG), :] + acc[L + M_MEM:2 * L]

        def b_pre(_):
            xa = jnp.concatenate([xs[pl.ds(r, SEG), :] for r, _v in ba_rows], axis=0)
            y = _ln(xa)
            for l in range(2):
                ybuf[pl.ds(ba_rows[l][0], SEG), :] = y[SEG * l:SEG * l + SEG] if l == 0 else ybuf_put(y)
            st['y2'] = _ln(y).astype(bf16)

        def ybuf_put(y):
            return y[SEG:2 * SEG]

        def b_mm1(_):
            hh = _gelu(_dot(st.pop('y2'), w1[...], NN))
            for l in range(2):
                hbuf[pl.ds(bah_rows[l], SEG), :] = hh[SEG * l:SEG * l + SEG]

        def b_shift(_):
            parts = []
            for l in range(2):
                win = hbuf[pl.ds(bbh_rows[l], SEG + 2 * HB_PAD), :]

                def sh(d, c):
                    return win[HB_PAD + d:HB_PAD + d + SEG, 128 * c:128 * c + 128]
                parts.append(jnp.concatenate([
                    sh(-1, 0),
                    jnp.where(lane32 < 32, sh(-1, 1), sh(1, 1)),
                    jnp.where(lane32 < 64, sh(1, 2), sh(-2, 2)),
                    jnp.where(lane32 < 96, sh(-2, 3), sh(2, 3)),
                    sh(2, 4)], axis=1))
            st['hsft'] = jnp.concatenate(parts, axis=0).astype(bf16)

        def b_mm2(_):
            hs = _dot(st.pop('hsft'), w2[...], NN)
            y = jnp.concatenate([ybuf[pl.ds(r, SEG), :] for r, _v in bb_rows], axis=0)
            x1 = y + hs
            xa = jnp.concatenate([xs[pl.ds(r, SEG), :] for r, _v in bb_rows], axis=0)
            st['res'] = xa + x1
            st['z'] = _ln(x1).astype(bf16)

        def b_mm3(c):
            st['g', c] = _gelu(_dot(st['z'], w3[:, pl.ds(512 * c, 512)], NN)).astype(bf16)

        def b_mm4(c):
            r = _dot(st.pop(('g', c)), w4[pl.ds(512 * c, 512), :], NN)
            st['res'] = st['res'] + r

        def b_fin(_):
            o = st.pop('res')
            o1 = o[0:SEG]
            xs[pl.ds(bb_rows[0][0], SEG), :] = o1
            lnx2[pl.ds(bb_rows[0][0], SEG), :] = _ln(o1)
            out_ref[pl.ds(out_row, SEG), :] = o[SEG:2 * SEG].astype(bf16)

        extra = {
            (-2, 'pre'): [(b_pre, 0)],
            (1, 'end'): [(b_mm1, 0)],
            (3, 'pre'): [(b_shift, 0)],
            (5, 'end'): [(b_mm2, 0)],
            (13, 'end'): [(b_mm3, 0)],
            (14, 's'): [],
            (14, 'out'): [(b_mm3, 1)],
            (14, 'pv'): [(b_mm3, 2)],
            (15, 'out'): [(a_fin, 0), (b_mm4, 0), (b_mm4, 1), (b_mm4, 2), (b_fin, 0)],
        }
        for i in range(-2, NP):
            sched = list(extra.get((i, 'pre'), []))
            for name, fn, p in [('k', a_k, i + 2), ('s', a_s, i + 1), ('out', a_out, i), ('q', a_q, i + 2),
                                ('pv', a_pv, i + 1), ('v', a_v, i + 2)]:
                if 0 <= p < NP:
                    sched.append((fn, p))
                    sched += extra.get((i, name), [])
            sched += extra.get((i, 'end'), [])
            for fn, p in sched:
                fn(p)
        assert not st.get('x'), st.keys()
        return carry

    lax.fori_loop(0, NSEG + LAG + 2, step, 0)


@functools.partial(jax.jit, static_argnames=("A_seg_len",))
def pallas_interleave_layers__memory_aug_recurrent_mem_tr__mixer_s_mlp__prompt_kernel(
        A_x, A_mem0, A_Wq, A_Wk, A_Wv, A_Wo, A_seg_len, B_x, B_w1, B_w2, B_w3, B_w4):
    del B_x
    assert A_seg_len == SEG and A_x.shape == (1, S_LEN, D) and A_Wq.shape == (D, H, E)
    x = A_x.reshape(S_LEN, D)
    mem0 = A_mem0.reshape(M_MEM, D)
    wqt, wkt, wvt = (jnp.transpose(w, (1, 2, 0)).reshape(H * E, D) for w in (A_Wq, A_Wk, A_Wv))
    wo = A_Wo.reshape(H * E, D)
    any_spec = pl.BlockSpec(memory_space=pl.ANY)
    out = pl.pallas_call(
        _kernel,
        out_shape=jax.ShapeDtypeStruct((S_LEN, D), bf16),
        in_specs=[any_spec, pl.BlockSpec(memory_space=pltpu.VMEM)] + [any_spec] * 8,
        out_specs=pl.BlockSpec(memory_space=pltpu.VMEM),
        scratch_shapes=[
            pltpu.VMEM((S_LEN, D), bf16),
            pltpu.VMEM((H * E, D), bf16), pltpu.VMEM((H * E, D), bf16),
            pltpu.VMEM((H * E, D), bf16), pltpu.VMEM((H * E, D), bf16),
            pltpu.VMEM((D, D), bf16), pltpu.VMEM((D, D), bf16),
            pltpu.VMEM((D, F), bf16), pltpu.VMEM((F, D), bf16),
            pltpu.VMEM((XS_ROWS, D), f32), pltpu.VMEM((XS_ROWS, D), f32),
            pltpu.VMEM((XS_ROWS, D), f32), pltpu.VMEM((XS_ROWS, D), f32),
            pltpu.VMEM((HB_ROWS, D), f32),
            pltpu.VMEM((2 * M_MEM, D), f32),
            pltpu.SemaphoreType.DMA((9,)),
        ],
        compiler_params=pltpu.CompilerParams(vmem_limit_bytes=120 * 1024 * 1024),
        name="mem_mixer",
    )(x, mem0, wqt, wkt, wvt, wo, B_w1, B_w2, B_w3, B_w4)
    return out.reshape(1, S_LEN, D)
```

```python
import functools

import jax
import jax.numpy as jnp
import numpy as np
from jax import lax
import jax.experimental.pallas as pl
import jax.experimental.pallas.tpu as pltpu

f32 = jnp.float32
bf16 = jnp.bfloat16

S_LEN, D, H, E = 2048, 640, 32, 192
M_MEM, SEG = 8, 32
L = M_MEM + SEG
NSEG = S_LEN // SEG
NP = H // 2
PW = 2 * E
F = 1536
LAG = 3
PREF = 3
EPS = 1e-5
NEG = -1e30

NT = (((1,), (1,)), ((), ()))
NN = (((1,), (0,)), ((), ()))


def _dot(a, b, dims):
    return lax.dot_general(a, b, dims, preferred_element_type=f32)


def _ln(x):
    m = jnp.mean(x, axis=-1, keepdims=True)
    xc = x - m
    v = jnp.mean(xc * xc, axis=-1, keepdims=True)
    return xc * lax.rsqrt(v + EPS)


def _gelu(x):
    c = np.float32(np.sqrt(2.0 / np.pi))
    return 0.5 * x * (1.0 + jnp.tanh(c * (x + np.float32(0.044715) * (x * x * x))))


XS_DUMMY = S_LEN
XS_ROWS = S_LEN + SEG
HB_PAD = 8
HB_DUMMY = S_LEN + 2 * HB_PAD
HB_ROWS = HB_DUMMY + SEG + 2 * HB_PAD

ORDER_V80 = {
    (-2, 'pre'): ['b_pre'],
    (1, 'end'): ['b_mm1'],
    (3, 'pre'): ['b_shift'],
    (5, 'end'): ['b_mm2'],
    (12, 'end'): ['b_mm3:0'],
    (13, 'end'): ['b_mm3:1'],
    (14, 's'): ['b_mm3:2'],
    (14, 'out'): ['b_mm4:0'],
    (14, 'pv'): ['b_mm4:1', 'b_mm4:2', 'b_fin'],
    (15, 'out'): ['a_fin'],
}
ORDER_V40 = ORDER_V80


def _kernel(x_hbm, mem0_ref, wq_hbm, wk_hbm, wv_hbm, wo_hbm, w1_hbm, w2_hbm, w3_hbm, w4_hbm,
            out_hbm,
            x_v, wq, wk, wv, wo, w1, w2, w3, w4, xs, lnx, ybuf, hbuf, mem, outs, sems, osem):
    def pair_copies(p):
        r = pl.ds(pl.multiple_of(p * PW, PW), PW)
        return [pltpu.make_async_copy(src.at[r], dst.at[r], sems.at[p])
                for src, dst in ((wk_hbm, wk), (wq_hbm, wq), (wv_hbm, wv), (wo_hbm, wo))]

    x_cp = pltpu.make_async_copy(x_hbm, x_v, sems.at[NP])
    b_cps = [pltpu.make_async_copy(src, dst, sems.at[NP + 1])
             for src, dst in ((w1_hbm, w1), (w2_hbm, w2), (w3_hbm, w3), (w4_hbm, w4))]
    x_cp.start()
    for p in range(PREF):
        for cp in pair_copies(p):
            cp.start()

    xs[pl.ds(XS_DUMMY, SEG), :] = jnp.zeros((SEG, D), f32)
    lnx[pl.ds(XS_DUMMY, SEG), :] = jnp.zeros((SEG, D), f32)
    ybuf[pl.ds(XS_DUMMY, SEG), :] = jnp.zeros((SEG, D), f32)
    hbuf[pl.ds(0, HB_PAD), :] = jnp.zeros((HB_PAD, D), f32)
    hbuf[pl.ds(HB_PAD + S_LEN, HB_ROWS - HB_PAD - S_LEN), :] = jnp.zeros((HB_ROWS - HB_PAD - S_LEN, D), f32)
    m0 = mem0_ref[...].astype(f32)
    mem[pl.ds(0, M_MEM), :] = m0
    mem[pl.ds(M_MEM, M_MEM), :] = m0
    x_cp.wait()

    def ln_init(s, c):
        r = pl.multiple_of(s * SEG, SEG)
        xf = x_v[pl.ds(r, SEG), :].astype(f32)
        xs[pl.ds(r, SEG), :] = xf
        lnx[pl.ds(r, SEG), :] = _ln(xf)
        return c
    lax.fori_loop(0, NSEG, ln_init, 0)

    lane128 = lax.broadcasted_iota(jnp.int32, (L, 128), 1)
    lo64 = lane128 < 64
    l80 = lax.broadcasted_iota(jnp.int32, (L, 2 * L), 1)
    row = lax.broadcasted_iota(jnp.int32, (L, 2 * L), 0)
    ha = l80 < L
    key = jnp.where(ha, l80, l80 - L)
    allowed = (row < M_MEM) | (row >= key)
    scale = np.float32(E ** -0.5)
    z40 = jnp.zeros((L, 128), f32)
    lane32 = lax.broadcasted_iota(jnp.int32, (SEG, 128), 1)

    def seg_row(seg, dummy=XS_DUMMY):
        valid = jnp.logical_and(seg >= 0, seg < NSEG)
        return pl.multiple_of(jnp.where(valid, seg * SEG, dummy), 8)

    def blk(u):
        t0 = jnp.concatenate([u[:, 0:128], z40], axis=0)
        u1 = u[:, 128:256]
        t1 = jnp.concatenate([jnp.where(lo64, u1, 0.), jnp.where(lo64, 0., u1)], axis=0)
        t2 = jnp.concatenate([z40, u[:, 256:384]], axis=0)
        return jnp.concatenate([t0, t1, t2], axis=1).astype(bf16)

    def softmax_parts(s):
        xm = jnp.where(allowed, s * scale, np.float32(-1e9))
        m0_ = jnp.max(jnp.where(ha, xm, NEG), axis=1, keepdims=True)
        m1_ = jnp.max(jnp.where(ha, NEG, xm), axis=1, keepdims=True)
        pe = jnp.exp(xm - jnp.where(ha, m0_, m1_))
        i0 = 1.0 / jnp.sum(jnp.where(ha, pe, 0.), axis=1, keepdims=True)
        i1 = 1.0 / jnp.sum(jnp.where(ha, 0., pe), axis=1, keepdims=True)
        return pe, i0, i1

    def pv(parts, vb):
        pe, i0, i1 = parts
        o = _dot(pe, vb, NN)
        return jnp.concatenate([o[:, 0:128] * i0, o[:, 128:256] * jnp.where(lo64, i0, i1), o[:, 256:384] * i1],
                               axis=1)

    def make_stages(a_slots, ba_segs, bb_slots):
        na = len(a_slots)
        st = {}
        a_rows = [seg_row(s) for s, _ in a_slots]
        ba_rows = [seg_row(s) for s in ba_segs]
        bb_rows = [seg_row(s) for s, _ in bb_slots]
        bah_rows = [seg_row(s, HB_DUMMY) + HB_PAD for s in ba_segs]
        bbh_rows = [seg_row(s, HB_DUMMY) for s, _ in bb_slots]
        fns = {}

        def stage(f):
            fns[f.__name__] = f
            return f

        if na:
            parts = []
            for (_, mr), r in zip(a_slots, a_rows):
                parts += [mem[pl.ds(mr, M_MEM), :], lnx[pl.ds(r, SEG), :]]
            h = jnp.concatenate(parts, axis=0).astype(bf16 if na == 2 else f32)

        def proj(w, p):
            return _dot(h, w[pl.ds(PW * p, PW), :], NT)

        @stage
        def a_k(p):
            k = proj(wk, p)
            st['k', p] = [blk(k[L * l:L * l + L]) for l in range(na)]

        @stage
        def a_q(p):
            q = proj(wq, p)
            st['q', p] = [q[L * l:L * l + L] for l in range(na)]

        @stage
        def a_v(p):
            v = proj(wv, p)
            st['v', p] = [blk(v[L * l:L * l + L]) for l in range(na)]

        @stage
        def a_s(p):
            qs, ks = st.pop(('q', p)), st.pop(('k', p))
            st['p', p] = [softmax_parts(_dot(qs[l], ks[l], NT)) for l in range(na)]

        @stage
        def a_pv(p):
            ps, vs = st.pop(('p', p)), st.pop(('v', p))
            o = jnp.concatenate([pv(ps[l], vs[l]) for l in range(na)], axis=0)
            st['o', p] = o.astype(bf16) if na == 2 else o

        @stage
        def a_out(p):
            r = _dot(st.pop(('o', p)), wo[pl.ds(PW * p, PW), :], NN)
            st['acc'] = r if 'acc' not in st else st['acc'] + r

        @stage
        def a_fin():
            acc = st.pop('acc')
            for l, ((_, mr), r) in enumerate(zip(a_slots, a_rows)):
                mem[pl.ds(mr, M_MEM), :] = acc[L * l:L * l + M_MEM]
                xs[pl.ds(r, SEG), :] = xs[pl.ds(r, SEG), :] + acc[L * l + M_MEM:L * l + L]

        @stage
        def b_pre():
            xa = jnp.concatenate([xs[pl.ds(r, SEG), :] for r in ba_rows], axis=0)
            y = _ln(xa)
            for l, r in enumerate(ba_rows):
                ybuf[pl.ds(r, SEG), :] = y[SEG * l:SEG * l + SEG]
            st['y2'] = _ln(y).astype(bf16)

        @stage
        def b_mm1():
            hh = _gelu(_dot(st.pop('y2'), w1[...], NN))
            for l, r in enumerate(bah_rows):
                hbuf[pl.ds(r, SEG), :] = hh[SEG * l:SEG * l + SEG]

        @stage
        def b_shift():
            parts = []
            for r in bbh_rows:
                win = hbuf[pl.ds(r, SEG + 2 * HB_PAD), :]

                def sh(d, c):
                    return win[HB_PAD + d:HB_PAD + d + SEG, 128 * c:128 * c + 128]
                parts.append(jnp.concatenate([
                    sh(-1, 0),
                    jnp.where(lane32 < 32, sh(-1, 1), sh(1, 1)),
                    jnp.where(lane32 < 64, sh(1, 2), sh(-2, 2)),
                    jnp.where(lane32 < 96, sh(-2, 3), sh(2, 3)),
                    sh(2, 4)], axis=1))
            st['hsft'] = jnp.concatenate(parts, axis=0).astype(bf16)

        @stage
        def b_mm2():
            hs = _dot(st.pop('hsft'), w2[...], NN)
            y = jnp.concatenate([ybuf[pl.ds(r, SEG), :] for r in bb_rows], axis=0)
            x1 = y + hs
            xa = jnp.concatenate([xs[pl.ds(r, SEG), :] for r in bb_rows], axis=0)
            st['res'] = xa + x1
            st['z'] = _ln(x1).astype(bf16)

        @stage
        def b_mm3(c):
            st['g', c] = _gelu(_dot(st['z'], w3[:, pl.ds(512 * c, 512)], NN)).astype(bf16)

        @stage
        def b_mm4(c):
            st['res'] = st['res'] + _dot(st.pop(('g', c)), w4[pl.ds(512 * c, 512), :], NN)

        @stage
        def b_fin():
            o = st.pop('res')
            for l, ((_, final), r) in enumerate(zip(bb_slots, bb_rows)):
                ol = o[SEG * l:SEG * l + SEG]
                if final:
                    outs[pl.ds(r, SEG), :] = ol.astype(bf16)
                else:
                    xs[pl.ds(r, SEG), :] = ol
                    lnx[pl.ds(r, SEG), :] = _ln(ol)

        def run(name):
            if ':' in name:
                n, a = name.split(':')
                fns[n](int(a))
            else:
                fns[name]()
        return run

    def run_order(run, order):
        for i in range(-2, NP):
            sched = list(order.get((i, 'pre'), []))
            for name, p in [('k', i + 2), ('s', i + 1), ('out', i), ('q', i + 2), ('pv', i + 1), ('v', i + 2)]:
                if 0 <= p < NP:
                    sched.append('a_%s:%d' % (name, p))
                    sched += order.get((i, name), [])
            sched += order.get((i, 'end'), [])
            for s in sched:
                run(s)

    def b_slots(t):
        return ([t - 1, t - LAG - 1], [(t - 2, False), (t - LAG - 2, True)])

    h0 = jnp.concatenate([mem[pl.ds(0, M_MEM), :], lnx[pl.ds(0, SEG), :]], axis=0)

    def first(p, acc):
        for cp in pair_copies(p):
            cp.wait()

        @pl.when(p + PREF < NP)
        def _():
            for cp in pair_copies(jnp.minimum(p + PREF, NP - 1)):
                cp.start()

        @pl.when(p + PREF == NP)
        def _():
            for cp in b_cps:
                cp.start()
        r = pl.ds(pl.multiple_of(p * PW, PW), PW)
        k = _dot(h0, wk[r, :], NT)
        q = _dot(h0, wq[r, :], NT)
        v = _dot(h0, wv[r, :], NT)
        o = pv(softmax_parts(_dot(q, blk(k), NT)), blk(v))
        return acc + _dot(o, wo[r, :], NN)
    acc0 = lax.fori_loop(0, NP, first, jnp.zeros((L, D), f32))
    mem[pl.ds(0, M_MEM), :] = acc0[0:M_MEM]
    xs[pl.ds(0, SEG), :] = xs[pl.ds(0, SEG), :] + acc0[M_MEM:L]
    for cp in b_cps:
        cp.wait()

    def step(t, carry):
        both = jnp.logical_and(t >= LAG, t < NSEG)

        @pl.when(both)
        def _():
            ba, bb = b_slots(t)
            run_order(make_stages([(t, 0), (t - LAG, M_MEM)], ba, bb), ORDER_V80)

        @pl.when(jnp.logical_not(both))
        def _():
            ba, bb = b_slots(t)
            early = t < LAG
            seg = jnp.where(early, t, t - LAG)
            mr = pl.multiple_of(jnp.where(early, 0, M_MEM), M_MEM)
            run_order(make_stages([(seg, mr)], ba, bb), ORDER_V40)
        return carry
    lax.fori_loop(1, NSEG + LAG, step, 0)

    n_done = NSEG - 2
    cp_a = pltpu.make_async_copy(outs.at[pl.ds(0, n_done * SEG)], out_hbm.at[pl.ds(0, n_done * SEG)], osem.at[0])
    cp_a.start()
    run = make_stages([], [NSEG - 1], [(NSEG - 2, True), (NSEG - 1, True)])
    for s in ['b_pre', 'b_mm1', 'b_shift', 'b_mm2', 'b_mm3:0', 'b_mm3:1', 'b_mm3:2', 'b_mm4:0', 'b_mm4:1', 'b_mm4:2',
              'b_fin']:
        run(s)
    cp_b = pltpu.make_async_copy(outs.at[pl.ds(n_done * SEG, 2 * SEG)], out_hbm.at[pl.ds(n_done * SEG, 2 * SEG)],
                                 osem.at[1])
    cp_b.start()
    cp_a.wait()
    cp_b.wait()


@functools.partial(jax.jit, static_argnames=("A_seg_len",))
def pallas_interleave_layers__memory_aug_recurrent_mem_tr__mixer_s_mlp__prompt_kernel(
        A_x, A_mem0, A_Wq, A_Wk, A_Wv, A_Wo, A_seg_len, B_x, B_w1, B_w2, B_w3, B_w4):
    del B_x
    assert A_seg_len == SEG and A_x.shape == (1, S_LEN, D) and A_Wq.shape == (D, H, E)
    x = A_x.reshape(S_LEN, D)
    mem0 = A_mem0.reshape(M_MEM, D)
    wqt, wkt, wvt = (jnp.transpose(w, (1, 2, 0)).reshape(H * E, D) for w in (A_Wq, A_Wk, A_Wv))
    wo = A_Wo.reshape(H * E, D)
    any_spec = pl.BlockSpec(memory_space=pl.ANY)
    out = pl.pallas_call(
        _kernel,
        out_shape=jax.ShapeDtypeStruct((S_LEN, D), bf16),
        in_specs=[any_spec, pl.BlockSpec(memory_space=pltpu.VMEM)] + [any_spec] * 8,
        out_specs=any_spec,
        scratch_shapes=[
            pltpu.VMEM((S_LEN, D), bf16),
            pltpu.VMEM((H * E, D), bf16), pltpu.VMEM((H * E, D), bf16),
            pltpu.VMEM((H * E, D), bf16), pltpu.VMEM((H * E, D), bf16),
            pltpu.VMEM((D, D), bf16), pltpu.VMEM((D, D), bf16),
            pltpu.VMEM((D, F), bf16), pltpu.VMEM((F, D), bf16),
            pltpu.VMEM((XS_ROWS, D), f32), pltpu.VMEM((XS_ROWS, D), f32),
            pltpu.VMEM((XS_ROWS, D), f32),
            pltpu.VMEM((HB_ROWS, D), f32),
            pltpu.VMEM((2 * M_MEM, D), f32),
            pltpu.VMEM((XS_ROWS, D), bf16),
            pltpu.SemaphoreType.DMA((NP + 2,)),
            pltpu.SemaphoreType.DMA((2,)),
        ],
        compiler_params=pltpu.CompilerParams(vmem_limit_bytes=120 * 1024 * 1024),
        name="mem_mixer",
    )(x, mem0, wqt, wkt, wvt, wo, B_w1, B_w2, B_w3, B_w4)
    return out.reshape(1, S_LEN, D)
```

```python
import functools

import jax
import jax.numpy as jnp
import numpy as np
from jax import lax
import jax.experimental.pallas as pl
import jax.experimental.pallas.tpu as pltpu

f32 = jnp.float32
bf16 = jnp.bfloat16

S_LEN, D, H, E = 2048, 640, 32, 192
M_MEM, SEG = 8, 32
L = M_MEM + SEG
NSEG = S_LEN // SEG
NP = H // 2
PW = 2 * E
F = 1536
LAG = 3
RING = 4
PRE0, NPRE = LAG, 7
PRE_ROWS = L + NPRE * SEG
EPS = 1e-5
NEG = -1e30

NT = (((1,), (1,)), ((), ()))
NN = (((1,), (0,)), ((), ()))


def _dot(a, b, dims):
    return lax.dot_general(a, b, dims, preferred_element_type=f32)


def _ln(x):
    m = jnp.mean(x, axis=-1, keepdims=True)
    xc = x - m
    v = jnp.mean(xc * xc, axis=-1, keepdims=True)
    return xc * lax.rsqrt(v + EPS)


def _gelu(x):
    c = np.float32(np.sqrt(2.0 / np.pi))
    return 0.5 * x * (1.0 + jnp.tanh(c * (x + np.float32(0.044715) * (x * x * x))))


XS_DUMMY = S_LEN
XS_ROWS = S_LEN + SEG
HB_PAD = 8
HB_DUMMY = S_LEN + 2 * HB_PAD
HB_ROWS = HB_DUMMY + SEG + 2 * HB_PAD

ORDER_V80 = {
    'iter': [('k', 2), ('q', 2), ('v', 2), ('s', 1), ('pv', 0), ('out', -1)],
    (-2, 'pre'): ['b_pre'], (1, 'end'): ['b_mm1'], (3, 'pre'): ['b_shift'], (5, 'end'): ['b_mm2'],
    (11, 'end'): ['b_mm3:0'], (12, 'end'): ['b_mm3:1'], (13, 'end'): ['b_mm3:2'], (14, 'end'): ['b_mm4:0'],
    (15, 'pv'): ['b_mm4:1'], (15, 'end'): ['b_mm4:2', 'b_fin'], (16, 'out'): ['a_fin'],
}
ORDER_V48 = ORDER_V80
ORDER_V40 = {
    'iter': [('k', 2), ('q', 2), ('v', 2), ('s', 1), ('pv', 0), ('out', -1)],
    (-2, 'pre'): ['b_pre'], (6, 'end'): ['b_wait'], (7, 'pre'): ['b_mm1'], (8, 'end'): ['b_shift', 'b_mm2'],
    (11, 'end'): ['b_mm3:0'], (12, 'end'): ['b_mm3:1'], (13, 'end'): ['b_mm3:2'], (14, 'end'): ['b_mm4:0'],
    (15, 'pv'): ['b_mm4:1'], (15, 'end'): ['b_mm4:2', 'b_fin'], (16, 'out'): ['a_fin'],
}


def _kernel(x_hbm, mem0_ref, wq_hbm, wk_hbm, wv_hbm, wo_hbm, w1_hbm, w2_hbm, w3_hbm, w4_hbm,
            out_hbm,
            x_v, stg, wn, won, w1, w2, w3, w4, xs, lnx, ybuf, hbuf, mem, outs, pre, sems, osem):
    def pair_copies(p):
        r = pl.ds(pl.multiple_of(p * PW, PW), PW)
        slot = p % RING
        return [pltpu.make_async_copy(src.at[r], stg.at[slot, m], sems.at[slot])
                for m, src in enumerate((wk_hbm, wq_hbm, wv_hbm, wo_hbm))]

    n0 = (PRE0 + NPRE) * SEG
    x_cp0 = pltpu.make_async_copy(x_hbm.at[pl.ds(0, n0)], x_v.at[pl.ds(0, n0)], sems.at[RING])
    x_cp = pltpu.make_async_copy(x_hbm.at[pl.ds(n0, S_LEN - n0)], x_v.at[pl.ds(n0, S_LEN - n0)], sems.at[RING + 1])
    b_cps = [pltpu.make_async_copy(src, dst, sems.at[RING + 2])
             for src, dst in ((w1_hbm, w1), (w2_hbm, w2), (w3_hbm, w3), (w4_hbm, w4))]
    x_cp0.start()
    for p in range(RING - 1):
        for cp in pair_copies(p):
            cp.start()
        if p == 0:
            x_cp.start()

    xs[pl.ds(XS_DUMMY, SEG), :] = jnp.zeros((SEG, D), f32)
    lnx[pl.ds(XS_DUMMY, SEG), :] = jnp.zeros((SEG, D), f32)
    ybuf[pl.ds(XS_DUMMY, SEG), :] = jnp.zeros((SEG, D), f32)
    hbuf[pl.ds(0, HB_PAD), :] = jnp.zeros((HB_PAD, D), f32)
    hbuf[pl.ds(HB_PAD + S_LEN, HB_ROWS - HB_PAD - S_LEN), :] = jnp.zeros((HB_ROWS - HB_PAD - S_LEN, D), f32)
    m0 = mem0_ref[...].astype(f32)
    mem[pl.ds(0, M_MEM), :] = m0
    mem[pl.ds(M_MEM, M_MEM), :] = m0
    x_cp0.wait()
    ln0 = _ln(x_v[pl.ds(0, n0), :].astype(f32))

    lane128 = lax.broadcasted_iota(jnp.int32, (L, 128), 1)
    lo64 = lane128 < 64
    l80 = lax.broadcasted_iota(jnp.int32, (L, 2 * L), 1)
    row = lax.broadcasted_iota(jnp.int32, (L, 2 * L), 0)
    ha = l80 < L
    key = jnp.where(ha, l80, l80 - L)
    allowed = (row < M_MEM) | (row >= key)
    scale = np.float32(E ** -0.5)
    z40 = jnp.zeros((L, 128), f32)
    lane32 = lax.broadcasted_iota(jnp.int32, (SEG, 128), 1)

    def seg_row(seg, dummy=XS_DUMMY):
        valid = jnp.logical_and(seg >= 0, seg < NSEG)
        return pl.multiple_of(jnp.where(valid, seg * SEG, dummy), 8)

    def blk(u):
        t0 = jnp.concatenate([u[:, 0:128], z40], axis=0)
        u1 = u[:, 128:256]
        t1 = jnp.concatenate([jnp.where(lo64, u1, 0.), jnp.where(lo64, 0., u1)], axis=0)
        t2 = jnp.concatenate([z40, u[:, 256:384]], axis=0)
        return jnp.concatenate([t0, t1, t2], axis=1).astype(bf16)

    def softmax_parts(s):
        xm = jnp.where(allowed, s * scale, np.float32(-1e9))
        m0_ = jnp.max(jnp.where(ha, xm, NEG), axis=1, keepdims=True)
        m1_ = jnp.max(jnp.where(ha, NEG, xm), axis=1, keepdims=True)
        pe = jnp.exp(xm - jnp.where(ha, m0_, m1_))
        i0 = 1.0 / jnp.sum(jnp.where(ha, pe, 0.), axis=1, keepdims=True)
        i1 = 1.0 / jnp.sum(jnp.where(ha, 0., pe), axis=1, keepdims=True)
        return pe, i0, i1

    def pv(parts, vb):
        pe, i0, i1 = parts
        o = _dot(pe, vb, NN)
        return jnp.concatenate([o[:, 0:128] * i0, o[:, 128:256] * jnp.where(lo64, i0, i1), o[:, 256:384] * i1],
                               axis=1)

    def make_stages(a_slots, ba_segs, bb_slots, pre_row=None, first_b=None):
        na = len(a_slots)
        st = {}
        a_rows = [seg_row(s) for s, _ in a_slots]
        ba_rows = [seg_row(s) for s in ba_segs]
        bb_rows = [seg_row(s) for s, _ in bb_slots]
        bah_rows = [seg_row(s, HB_DUMMY) + HB_PAD for s in ba_segs]
        bbh_rows = [seg_row(s, HB_DUMMY) for s, _ in bb_slots]
        fns = {}

        def stage(f):
            fns[f.__name__] = f
            return f

        if na:
            parts = []
            for l, ((_, mr), r) in enumerate(zip(a_slots, a_rows)):
                parts.append(mem[pl.ds(mr, M_MEM), :])
                if not (l == 0 and pre_row is not None):
                    parts.append(lnx[pl.ds(r, SEG), :])
            h = jnp.concatenate(parts, axis=0).astype(bf16 if na == 2 else f32)

        def proj(m, p):
            r = _dot(h, pltpu.bitcast(wn[p, m], bf16), NN)
            if pre_row is None:
                return [r[L * l:L * l + L] for l in range(na)]
            tok = pre[m, pl.ds(pre_row, SEG), pl.ds(PW * p, PW)]
            return [jnp.concatenate([r[0:M_MEM], tok], axis=0), r[M_MEM:M_MEM + L]]

        @stage
        def a_k(p):
            st['k', p] = [blk(k) for k in proj(0, p)]

        @stage
        def a_q(p):
            st['q', p] = proj(1, p)

        @stage
        def a_v(p):
            st['v', p] = [blk(v) for v in proj(2, p)]

        @stage
        def a_s(p):
            qs, ks = st.pop(('q', p)), st.pop(('k', p))
            st['p', p] = [softmax_parts(_dot(qs[l], ks[l], NT)) for l in range(na)]

        @stage
        def a_pv(p):
            ps, vs = st.pop(('p', p)), st.pop(('v', p))
            o = jnp.concatenate([pv(ps[l], vs[l]) for l in range(na)], axis=0)
            st['o', p] = o.astype(bf16) if na == 2 else o

        @stage
        def a_out(p):
            r = _dot(st.pop(('o', p)), pltpu.bitcast(won[p], bf16), NN)
            st['acc'] = r if 'acc' not in st else st['acc'] + r

        @stage
        def a_fin():
            acc = st.pop('acc')
            for l, ((_, mr), r) in enumerate(zip(a_slots, a_rows)):
                mem[pl.ds(mr, M_MEM), :] = acc[L * l:L * l + M_MEM]
                xs[pl.ds(r, SEG), :] = xs[pl.ds(r, SEG), :] + acc[L * l + M_MEM:L * l + L]

        @stage
        def b_wait():
            @pl.when(first_b)
            def _():
                for cp in b_cps:
                    cp.wait()

        @stage
        def b_pre():
            xa = jnp.concatenate([xs[pl.ds(r, SEG), :] for r in ba_rows], axis=0)
            y = _ln(xa)
            for l, r in enumerate(ba_rows):
                ybuf[pl.ds(r, SEG), :] = y[SEG * l:SEG * l + SEG]
            st['y2'] = _ln(y).astype(bf16)

        @stage
        def b_mm1():
            hh = _gelu(_dot(st.pop('y2'), w1[...], NN))
            for l, r in enumerate(bah_rows):
                hbuf[pl.ds(r, SEG), :] = hh[SEG * l:SEG * l + SEG]

        @stage
        def b_shift():
            parts = []
            for r in bbh_rows:
                win = hbuf[pl.ds(r, SEG + 2 * HB_PAD), :]

                def sh(d, c):
                    return win[HB_PAD + d:HB_PAD + d + SEG, 128 * c:128 * c + 128]
                parts.append(jnp.concatenate([
                    sh(-1, 0),
                    jnp.where(lane32 < 32, sh(-1, 1), sh(1, 1)),
                    jnp.where(lane32 < 64, sh(1, 2), sh(-2, 2)),
                    jnp.where(lane32 < 96, sh(-2, 3), sh(2, 3)),
                    sh(2, 4)], axis=1))
            st['hsft'] = jnp.concatenate(parts, axis=0).astype(bf16)

        @stage
        def b_mm2():
            hs = _dot(st.pop('hsft'), w2[...], NN)
            y = jnp.concatenate([ybuf[pl.ds(r, SEG), :] for r in bb_rows], axis=0)
            x1 = y + hs
            xa = jnp.concatenate([xs[pl.ds(r, SEG), :] for r in bb_rows], axis=0)
            st['res'] = xa + x1
            st['z'] = _ln(x1).astype(bf16)

        @stage
        def b_mm3(c):
            st['g', c] = _gelu(_dot(st['z'], w3[:, pl.ds(512 * c, 512)], NN)).astype(bf16)

        @stage
        def b_mm4(c):
            st['res'] = st['res'] + _dot(st.pop(('g', c)), w4[pl.ds(512 * c, 512), :], NN)

        @stage
        def b_fin():
            o = st.pop('res')
            for l, ((_, final), r) in enumerate(zip(bb_slots, bb_rows)):
                ol = o[SEG * l:SEG * l + SEG]
                if final:
                    outs[pl.ds(r, SEG), :] = ol.astype(bf16)
                else:
                    xs[pl.ds(r, SEG), :] = ol
                    lnx[pl.ds(r, SEG), :] = _ln(ol)

        def run(name):
            if ':' in name:
                n, a = name.split(':')
                fns[n](int(a))
            else:
                fns[name]()
        return run

    def run_order(run, order):
        offs = [o for _, o in order['iter']]
        for i in range(-max(offs), NP - min(offs)):
            sched = list(order.get((i, 'pre'), []))
            for name, o in order['iter']:
                if 0 <= i + o < NP:
                    sched.append('a_%s:%d' % (name, i + o))
                    sched += order.get((i, name), [])
            sched += order.get((i, 'end'), [])
            for s in sched:
                run(s)

    def b_slots(t):
        return ([t - 1, t - LAG - 1], [(t - 2, False), (t - LAG - 2, True)])

    h0 = jnp.concatenate([m0, ln0[0:SEG], ln0[PRE0 * SEG:n0]], axis=0)
    x_cp.wait()
    nl = S_LEN // NP

    def attend0(p):
        c = pl.ds(pl.multiple_of(p * PW, PW), PW)
        st = {}

        def a_s():
            st['p'] = softmax_parts(_dot(pre[1, pl.ds(0, L), c], blk(pre[0, pl.ds(0, L), c]), NT))

        def a_pv():
            st['o'] = pv(st['p'], blk(pre[2, pl.ds(0, L), c]))

        def a_out(acc):
            return acc + _dot(st['o'], pltpu.bitcast(won[p], bf16), NN)
        return a_s, a_pv, a_out

    for m in range(3):
        pre[m, pl.ds(0, L), pl.ds(0, PW)] = jnp.zeros((L, PW), f32)

    def first(p, acc):
        @pl.when(p + RING - 1 < NP)
        def _():
            for cp in pair_copies(jnp.minimum(p + RING - 1, NP - 1)):
                cp.start()

        @pl.when(p + RING - 1 == NP)
        def _():
            for cp in b_cps:
                cp.start()
        for cp in pair_copies(p):
            cp.wait()
        slot = p % RING
        c = pl.ds(pl.multiple_of(p * PW, PW), PW)
        a_s, a_pv, a_out = attend0(jnp.maximum(p - 1, 0))

        def proj0(m):
            w = stg[slot, m]
            wn[p, m] = pltpu.bitcast(jnp.transpose(w), jnp.uint32)
            return _dot(h0, w, NT)
        won[p] = pltpu.bitcast(stg[slot, 3], jnp.uint32)
        k = proj0(0)
        a_s()
        pre_q = proj0(1)
        a_pv()
        pre[0, :, c] = k
        pre[1, :, c] = pre_q
        rr = pl.ds(pl.multiple_of(p * nl, nl), nl)
        xf = x_v[rr, :].astype(f32)
        xs[rr, :] = xf
        lnx[rr, :] = _ln(xf)
        acc = a_out(acc)
        pre[2, :, c] = proj0(2)
        return acc
    acc0 = lax.fori_loop(0, NP, first, jnp.zeros((L, D), f32))
    a_s, a_pv, a_out = attend0(NP - 1)
    a_s()
    a_pv()
    acc0 = a_out(acc0)
    mem[pl.ds(0, M_MEM), :] = acc0[0:M_MEM]
    xs[pl.ds(0, SEG), :] = xs[pl.ds(0, SEG), :] + acc0[M_MEM:L]

    def step(t, carry):
        pre_on = jnp.logical_and(t >= PRE0, t < PRE0 + NPRE)
        full = jnp.logical_and(t >= PRE0 + NPRE, t < NSEG)
        single = jnp.logical_or(t < LAG, t >= NSEG)

        @pl.when(full)
        def _():
            ba, bb = b_slots(t)
            run_order(make_stages([(t, 0), (t - LAG, M_MEM)], ba, bb), ORDER_V80)

        @pl.when(pre_on)
        def _():
            ba, bb = b_slots(t)
            pr = pl.multiple_of(L + (jnp.clip(t, PRE0, PRE0 + NPRE - 1) - PRE0) * SEG, 8)
            run_order(make_stages([(t, 0), (t - LAG, M_MEM)], ba, bb, pre_row=pr), ORDER_V48)

        @pl.when(single)
        def _():
            ba, bb = b_slots(t)
            early = t < LAG
            seg = jnp.where(early, t, t - LAG)
            mr = pl.multiple_of(jnp.where(early, 0, M_MEM), M_MEM)
            run_order(make_stages([(seg, mr)], ba, bb, first_b=(t == 1)), ORDER_V40)
        return carry
    lax.fori_loop(1, NSEG + LAG, step, 0)

    n_done = NSEG - 2
    cp_a = pltpu.make_async_copy(outs.at[pl.ds(0, n_done * SEG)], out_hbm.at[pl.ds(0, n_done * SEG)], osem.at[0])
    cp_a.start()
    run = make_stages([], [NSEG - 1], [(NSEG - 2, True), (NSEG - 1, True)])
    for s in ['b_pre', 'b_mm1', 'b_shift', 'b_mm2', 'b_mm3:0', 'b_mm3:1', 'b_mm3:2', 'b_mm4:0', 'b_mm4:1', 'b_mm4:2',
              'b_fin']:
        run(s)
    cp_b = pltpu.make_async_copy(outs.at[pl.ds(n_done * SEG, 2 * SEG)], out_hbm.at[pl.ds(n_done * SEG, 2 * SEG)],
                                 osem.at[1])
    cp_b.start()
    cp_a.wait()
    cp_b.wait()


@functools.partial(jax.jit, static_argnames=("A_seg_len",))
def pallas_interleave_layers__memory_aug_recurrent_mem_tr__mixer_s_mlp__prompt_kernel(
        A_x, A_mem0, A_Wq, A_Wk, A_Wv, A_Wo, A_seg_len, B_x, B_w1, B_w2, B_w3, B_w4):
    del B_x
    assert A_seg_len == SEG and A_x.shape == (1, S_LEN, D) and A_Wq.shape == (D, H, E)
    x = A_x.reshape(S_LEN, D)
    mem0 = A_mem0.reshape(M_MEM, D)
    wqt, wkt, wvt = (jnp.transpose(w, (1, 2, 0)).reshape(H * E, D) for w in (A_Wq, A_Wk, A_Wv))
    wo = A_Wo.reshape(H * E, D)
    any_spec = pl.BlockSpec(memory_space=pl.ANY)
    out = pl.pallas_call(
        _kernel,
        out_shape=jax.ShapeDtypeStruct((S_LEN, D), bf16),
        in_specs=[any_spec, pl.BlockSpec(memory_space=pltpu.VMEM)] + [any_spec] * 8,
        out_specs=any_spec,
        scratch_shapes=[
            pltpu.VMEM((S_LEN, D), bf16),
            pltpu.VMEM((RING, 4, PW, D), bf16),
            pltpu.VMEM((NP, 3, D // 2, PW), jnp.uint32),
            pltpu.VMEM((NP, PW // 2, D), jnp.uint32),
            pltpu.VMEM((D, D), bf16), pltpu.VMEM((D, D), bf16),
            pltpu.VMEM((D, F), bf16), pltpu.VMEM((F, D), bf16),
            pltpu.VMEM((XS_ROWS, D), f32), pltpu.VMEM((XS_ROWS, D), f32),
            pltpu.VMEM((XS_ROWS, D), f32),
            pltpu.VMEM((HB_ROWS, D), f32),
            pltpu.VMEM((2 * M_MEM, D), f32),
            pltpu.VMEM((XS_ROWS, D), bf16),
            pltpu.VMEM((3, PRE_ROWS, H * E), f32),
            pltpu.SemaphoreType.DMA((RING + 3,)),
            pltpu.SemaphoreType.DMA((2,)),
        ],
        compiler_params=pltpu.CompilerParams(vmem_limit_bytes=120 * 1024 * 1024),
        name="mem_mixer",
    )(x, mem0, wqt, wkt, wvt, wo, B_w1, B_w2, B_w3, B_w4)
    return out.reshape(1, S_LEN, D)
```

```python
import functools

import jax
import jax.numpy as jnp
import numpy as np
from jax import lax
import jax.experimental.pallas as pl
import jax.experimental.pallas.tpu as pltpu

f32 = jnp.float32
bf16 = jnp.bfloat16

S_LEN, D, H, E = 2048, 640, 32, 192
M_MEM, SEG = 8, 32
L = M_MEM + SEG
NSEG = S_LEN // SEG
NP = H // 2
PW = 2 * E
F = 1536
LAG = 3
RING = 4
PRE0, NPRE = LAG, 8
PRE_ROWS = L + NPRE * SEG
EPS = 1e-5
NEG = -1e30

NT = (((1,), (1,)), ((), ()))
NN = (((1,), (0,)), ((), ()))


def _dot(a, b, dims):
    return lax.dot_general(a, b, dims, preferred_element_type=f32)


def _ln(x):
    m = jnp.mean(x, axis=-1, keepdims=True)
    xc = x - m
    v = jnp.mean(xc * xc, axis=-1, keepdims=True)
    return xc * lax.rsqrt(v + EPS)


def _gelu(x):
    c = np.float32(np.sqrt(2.0 / np.pi))
    return 0.5 * x * (1.0 + jnp.tanh(c * (x + np.float32(0.044715) * (x * x * x))))


XS_DUMMY = S_LEN
XS_ROWS = S_LEN + SEG
HB_PAD = 8
HB_DUMMY = S_LEN + 2 * HB_PAD
HB_ROWS = HB_DUMMY + SEG + 2 * HB_PAD

ORDER_V80 = {
    'iter': [('k', 2), ('q', 2), ('v', 2), ('s', 1), ('pv', 0), ('out', -1)],
    (-2, 'pre'): ['b_pre'], (1, 'end'): ['b_mm1'], (3, 'pre'): ['b_shift'], (5, 'end'): ['b_mm2'],
    (8, 'pre'): ['x_ln'],
    (11, 'end'): ['b_mm3:0'], (12, 'end'): ['b_mm3:1'], (13, 'end'): ['b_mm3:2'], (14, 'end'): ['b_mm4:0'],
    (15, 'pv'): ['b_mm4:1'], (15, 'end'): ['b_mm4:2', 'b_fin'], (16, 'out'): ['a_fin'],
}
ORDER_V48 = ORDER_V80
ORDER_V40 = {
    'iter': [('k', 2), ('q', 2), ('v', 2), ('s', 1), ('pv', 0), ('out', -1)],
    (-2, 'pre'): ['b_pre'], (6, 'end'): ['b_wait'], (7, 'pre'): ['b_mm1'], (8, 'end'): ['b_shift', 'b_mm2'],
    (11, 'end'): ['b_mm3:0'], (12, 'end'): ['b_mm3:1'], (13, 'end'): ['b_mm3:2'], (14, 'end'): ['b_mm4:0'],
    (15, 'pv'): ['b_mm4:1'], (15, 'end'): ['b_mm4:2', 'b_fin'], (16, 'out'): ['a_fin'],
}


def _kernel(x_hbm, mem0_ref, wq_hbm, wk_hbm, wv_hbm, wo_hbm, w1_hbm, w2_hbm, w3_hbm, w4_hbm,
            out_hbm,
            x_v, stg, wn, won, w1, w2, w3, w4, xs, lnx, ybuf, hbuf, mem, outs, pre, sems, osem):
    def pair_copies(p):
        r = pl.ds(pl.multiple_of(p * PW, PW), PW)
        slot = p % RING
        return [pltpu.make_async_copy(src.at[r], stg.at[slot, m], sems.at[slot])
                for m, src in enumerate((wk_hbm, wq_hbm, wv_hbm, wo_hbm))]

    n0 = (PRE0 + NPRE) * SEG
    x_cp0 = pltpu.make_async_copy(x_hbm.at[pl.ds(0, n0)], x_v.at[pl.ds(0, n0)], sems.at[RING])
    x_cp = pltpu.make_async_copy(x_hbm.at[pl.ds(n0, S_LEN - n0)], x_v.at[pl.ds(n0, S_LEN - n0)], sems.at[RING + 1])
    b_cps = [pltpu.make_async_copy(src, dst, sems.at[RING + 2])
             for src, dst in ((w1_hbm, w1), (w2_hbm, w2), (w3_hbm, w3), (w4_hbm, w4))]
    x_cp0.start()
    for p in range(RING - 1):
        for cp in pair_copies(p):
            cp.start()

    xs[pl.ds(XS_DUMMY, SEG), :] = jnp.zeros((SEG, D), f32)
    lnx[pl.ds(XS_DUMMY, SEG), :] = jnp.zeros((SEG, D), f32)
    ybuf[pl.ds(XS_DUMMY, SEG), :] = jnp.zeros((SEG, D), f32)
    hbuf[pl.ds(0, HB_PAD), :] = jnp.zeros((HB_PAD, D), f32)
    hbuf[pl.ds(HB_PAD + S_LEN, HB_ROWS - HB_PAD - S_LEN), :] = jnp.zeros((HB_ROWS - HB_PAD - S_LEN, D), f32)
    m0 = mem0_ref[...].astype(f32)
    mem[pl.ds(0, M_MEM), :] = m0
    mem[pl.ds(M_MEM, M_MEM), :] = m0
    x_cp0.wait()
    xf0 = x_v[pl.ds(0, n0), :].astype(f32)
    ln0 = _ln(xf0)
    xs[pl.ds(0, n0), :] = xf0
    lnx[pl.ds(0, n0), :] = ln0

    lane128 = lax.broadcasted_iota(jnp.int32, (L, 128), 1)
    lo64 = lane128 < 64
    l80 = lax.broadcasted_iota(jnp.int32, (L, 2 * L), 1)
    row = lax.broadcasted_iota(jnp.int32, (L, 2 * L), 0)
    ha = l80 < L
    key = jnp.where(ha, l80, l80 - L)
    allowed = (row < M_MEM) | (row >= key)
    scale = np.float32(E ** -0.5)
    z40 = jnp.zeros((L, 128), f32)
    lane32 = lax.broadcasted_iota(jnp.int32, (SEG, 128), 1)

    def seg_row(seg, dummy=XS_DUMMY):
        valid = jnp.logical_and(seg >= 0, seg < NSEG)
        return pl.multiple_of(jnp.where(valid, seg * SEG, dummy), 8)

    def blk(u):
        t0 = jnp.concatenate([u[:, 0:128], z40], axis=0)
        u1 = u[:, 128:256]
        t1 = jnp.concatenate([jnp.where(lo64, u1, 0.), jnp.where(lo64, 0., u1)], axis=0)
        t2 = jnp.concatenate([z40, u[:, 256:384]], axis=0)
        return jnp.concatenate([t0, t1, t2], axis=1).astype(bf16)

    def softmax_parts(s):
        xm = jnp.where(allowed, s * scale, np.float32(-1e9))
        m0_ = jnp.max(jnp.where(ha, xm, NEG), axis=1, keepdims=True)
        m1_ = jnp.max(jnp.where(ha, NEG, xm), axis=1, keepdims=True)
        pe = jnp.exp(xm - jnp.where(ha, m0_, m1_))
        i0 = 1.0 / jnp.sum(jnp.where(ha, pe, 0.), axis=1, keepdims=True)
        i1 = 1.0 / jnp.sum(jnp.where(ha, 0., pe), axis=1, keepdims=True)
        return pe, i0, i1

    def pv(parts, vb):
        pe, i0, i1 = parts
        o = _dot(pe, vb, NN)
        return jnp.concatenate([o[:, 0:128] * i0, o[:, 128:256] * jnp.where(lo64, i0, i1), o[:, 256:384] * i1],
                               axis=1)

    def make_stages(a_slots, ba_segs, bb_slots, pre_row=None, first_b=None):
        na = len(a_slots)
        st = {}
        a_rows = [seg_row(s) for s, _ in a_slots]
        ba_rows = [seg_row(s) for s in ba_segs]
        bb_rows = [seg_row(s) for s, _ in bb_slots]
        bah_rows = [seg_row(s, HB_DUMMY) + HB_PAD for s in ba_segs]
        bbh_rows = [seg_row(s, HB_DUMMY) for s, _ in bb_slots]
        fns = {}

        def stage(f):
            fns[f.__name__] = f
            return f

        if na:
            parts = []
            for l, ((_, mr), r) in enumerate(zip(a_slots, a_rows)):
                parts.append(mem[pl.ds(mr, M_MEM), :])
                if not (l == 0 and pre_row is not None):
                    parts.append(lnx[pl.ds(r, SEG), :])
            h = jnp.concatenate(parts, axis=0).astype(bf16 if na == 2 else f32)

        def proj(m, p):
            r = _dot(h, pltpu.bitcast(wn[p, m], bf16), NN)
            if pre_row is None:
                return [r[L * l:L * l + L] for l in range(na)]
            tok = pre[m, pl.ds(pre_row, SEG), pl.ds(PW * p, PW)]
            return [jnp.concatenate([r[0:M_MEM], tok], axis=0), r[M_MEM:M_MEM + L]]

        @stage
        def a_k(p):
            st['k', p] = [blk(k) for k in proj(0, p)]

        @stage
        def a_q(p):
            st['q', p] = proj(1, p)

        @stage
        def a_v(p):
            st['v', p] = [blk(v) for v in proj(2, p)]

        @stage
        def a_s(p):
            qs, ks = st.pop(('q', p)), st.pop(('k', p))
            st['p', p] = [softmax_parts(_dot(qs[l], ks[l], NT)) for l in range(na)]

        @stage
        def a_pv(p):
            ps, vs = st.pop(('p', p)), st.pop(('v', p))
            o = jnp.concatenate([pv(ps[l], vs[l]) for l in range(na)], axis=0)
            st['o', p] = o.astype(bf16) if na == 2 else o

        @stage
        def a_out(p):
            r = _dot(st.pop(('o', p)), pltpu.bitcast(won[p], bf16), NN)
            st['acc'] = r if 'acc' not in st else st['acc'] + r

        @stage
        def a_fin():
            acc = st.pop('acc')
            for l, ((_, mr), r) in enumerate(zip(a_slots, a_rows)):
                mem[pl.ds(mr, M_MEM), :] = acc[L * l:L * l + M_MEM]
                xs[pl.ds(r, SEG), :] = xs[pl.ds(r, SEG), :] + acc[L * l + M_MEM:L * l + L]

        @stage
        def x_ln():
            seg = a_slots[0][0] + NPRE
            src = pl.multiple_of(jnp.minimum(seg, NSEG - 1) * SEG, SEG)
            xf = x_v[pl.ds(src, SEG), :].astype(f32)
            r = seg_row(seg)
            xs[pl.ds(r, SEG), :] = xf
            lnx[pl.ds(r, SEG), :] = _ln(xf)

        @stage
        def b_wait():
            @pl.when(first_b)
            def _():
                for cp in b_cps:
                    cp.wait()

        @stage
        def b_pre():
            xa = jnp.concatenate([xs[pl.ds(r, SEG), :] for r in ba_rows], axis=0)
            y = _ln(xa)
            for l, r in enumerate(ba_rows):
                ybuf[pl.ds(r, SEG), :] = y[SEG * l:SEG * l + SEG]
            st['y2'] = _ln(y).astype(bf16)

        @stage
        def b_mm1():
            hh = _gelu(_dot(st.pop('y2'), w1[...], NN))
            for l, r in enumerate(bah_rows):
                hbuf[pl.ds(r, SEG), :] = hh[SEG * l:SEG * l + SEG]

        @stage
        def b_shift():
            parts = []
            for r in bbh_rows:
                win = hbuf[pl.ds(r, SEG + 2 * HB_PAD), :]

                def sh(d, c):
                    return win[HB_PAD + d:HB_PAD + d + SEG, 128 * c:128 * c + 128]
                parts.append(jnp.concatenate([
                    sh(-1, 0),
                    jnp.where(lane32 < 32, sh(-1, 1), sh(1, 1)),
                    jnp.where(lane32 < 64, sh(1, 2), sh(-2, 2)),
                    jnp.where(lane32 < 96, sh(-2, 3), sh(2, 3)),
                    sh(2, 4)], axis=1))
            st['hsft'] = jnp.concatenate(parts, axis=0).astype(bf16)

        @stage
        def b_mm2():
            hs = _dot(st.pop('hsft'), w2[...], NN)
            y = jnp.concatenate([ybuf[pl.ds(r, SEG), :] for r in bb_rows], axis=0)
            x1 = y + hs
            xa = jnp.concatenate([xs[pl.ds(r, SEG), :] for r in bb_rows], axis=0)
            st['res'] = xa + x1
            st['z'] = _ln(x1).astype(bf16)

        @stage
        def b_mm3(c):
            st['g', c] = _gelu(_dot(st['z'], w3[:, pl.ds(512 * c, 512)], NN)).astype(bf16)

        @stage
        def b_mm4(c):
            st['res'] = st['res'] + _dot(st.pop(('g', c)), w4[pl.ds(512 * c, 512), :], NN)

        @stage
        def b_fin():
            o = st.pop('res')
            for l, ((_, final), r) in enumerate(zip(bb_slots, bb_rows)):
                ol = o[SEG * l:SEG * l + SEG]
                if final:
                    outs[pl.ds(r, SEG), :] = ol.astype(bf16)
                else:
                    xs[pl.ds(r, SEG), :] = ol
                    lnx[pl.ds(r, SEG), :] = _ln(ol)

        def run(name):
            if ':' in name:
                n, a = name.split(':')
                fns[n](int(a))
            else:
                fns[name]()
        return run

    def run_order(run, order):
        offs = [o for _, o in order['iter']]
        for i in range(-max(offs), NP - min(offs)):
            sched = list(order.get((i, 'pre'), []))
            for name, o in order['iter']:
                if 0 <= i + o < NP:
                    sched.append('a_%s:%d' % (name, i + o))
                    sched += order.get((i, name), [])
            sched += order.get((i, 'end'), [])
            for s in sched:
                run(s)

    def b_slots(t):
        return ([t - 1, t - LAG - 1], [(t - 2, False), (t - LAG - 2, True)])

    h0 = jnp.concatenate([m0, ln0[0:SEG], ln0[PRE0 * SEG:n0]], axis=0)

    def attend0(p):
        c = pl.ds(pl.multiple_of(p * PW, PW), PW)
        st = {}

        def a_s():
            st['p'] = softmax_parts(_dot(pre[1, pl.ds(0, L), c], blk(pre[0, pl.ds(0, L), c]), NT))

        def a_pv():
            st['o'] = pv(st['p'], blk(pre[2, pl.ds(0, L), c]))

        def a_out(acc):
            return acc + _dot(st['o'], pltpu.bitcast(won[p], bf16), NN)
        return a_s, a_pv, a_out

    for m in range(3):
        pre[m, pl.ds(0, L), pl.ds(0, PW)] = jnp.zeros((L, PW), f32)

    def first(p, acc):
        @pl.when(p + RING - 1 < NP)
        def _():
            for cp in pair_copies(jnp.minimum(p + RING - 1, NP - 1)):
                cp.start()

        @pl.when(p + RING - 1 == NP)
        def _():
            for cp in b_cps:
                cp.start()
            x_cp.start()
        for cp in pair_copies(p):
            cp.wait()
        slot = p % RING
        c = pl.ds(pl.multiple_of(p * PW, PW), PW)
        a_s, a_pv, a_out = attend0(jnp.maximum(p - 1, 0))

        def proj0(m):
            w = stg[slot, m]
            wn[p, m] = pltpu.bitcast(jnp.transpose(w), jnp.uint32)
            return _dot(h0, w, NT)
        won[p] = pltpu.bitcast(stg[slot, 3], jnp.uint32)
        k = proj0(0)
        a_s()
        pre_q = proj0(1)
        a_pv()
        pre[0, :, c] = k
        pre[1, :, c] = pre_q
        v = proj0(2)
        acc = a_out(acc)
        pre[2, :, c] = v
        return acc
    acc0 = lax.fori_loop(0, NP, first, jnp.zeros((L, D), f32))
    a_s, a_pv, a_out = attend0(NP - 1)
    a_s()
    a_pv()
    acc0 = a_out(acc0)
    mem[pl.ds(0, M_MEM), :] = acc0[0:M_MEM]
    xs[pl.ds(0, SEG), :] = xs[pl.ds(0, SEG), :] + acc0[M_MEM:L]

    def step(t, carry):
        pre_on = jnp.logical_and(t >= PRE0, t < PRE0 + NPRE)
        full = jnp.logical_and(t >= PRE0 + NPRE, t < NSEG)
        single = jnp.logical_or(t < LAG, t >= NSEG)

        @pl.when(t == LAG)
        def _():
            x_cp.wait()

        @pl.when(full)
        def _():
            ba, bb = b_slots(t)
            run_order(make_stages([(t, 0), (t - LAG, M_MEM)], ba, bb), ORDER_V80)

        @pl.when(pre_on)
        def _():
            ba, bb = b_slots(t)
            pr = pl.multiple_of(L + (jnp.clip(t, PRE0, PRE0 + NPRE - 1) - PRE0) * SEG, 8)
            run_order(make_stages([(t, 0), (t - LAG, M_MEM)], ba, bb, pre_row=pr), ORDER_V48)

        @pl.when(single)
        def _():
            ba, bb = b_slots(t)
            early = t < LAG
            seg = jnp.where(early, t, t - LAG)
            mr = pl.multiple_of(jnp.where(early, 0, M_MEM), M_MEM)
            run_order(make_stages([(seg, mr)], ba, bb, first_b=(t == 1)), ORDER_V40)
        return carry
    lax.fori_loop(1, NSEG + LAG, step, 0)

    n_done = NSEG - 2
    cp_a = pltpu.make_async_copy(outs.at[pl.ds(0, n_done * SEG)], out_hbm.at[pl.ds(0, n_done * SEG)], osem.at[0])
    cp_a.start()
    run = make_stages([], [NSEG - 1], [(NSEG - 2, True), (NSEG - 1, True)])
    for s in ['b_pre', 'b_mm1', 'b_shift', 'b_mm2', 'b_mm3:0', 'b_mm3:1', 'b_mm3:2', 'b_mm4:0', 'b_mm4:1', 'b_mm4:2',
              'b_fin']:
        run(s)
    cp_b = pltpu.make_async_copy(outs.at[pl.ds(n_done * SEG, 2 * SEG)], out_hbm.at[pl.ds(n_done * SEG, 2 * SEG)],
                                 osem.at[1])
    cp_b.start()
    cp_a.wait()
    cp_b.wait()


@functools.partial(jax.jit, static_argnames=("A_seg_len",))
def pallas_interleave_layers__memory_aug_recurrent_mem_tr__mixer_s_mlp__prompt_kernel(
        A_x, A_mem0, A_Wq, A_Wk, A_Wv, A_Wo, A_seg_len, B_x, B_w1, B_w2, B_w3, B_w4):
    del B_x
    assert A_seg_len == SEG and A_x.shape == (1, S_LEN, D) and A_Wq.shape == (D, H, E)
    x = A_x.reshape(S_LEN, D)
    mem0 = A_mem0.reshape(M_MEM, D)
    wqt, wkt, wvt = (jnp.transpose(w, (1, 2, 0)).reshape(H * E, D) for w in (A_Wq, A_Wk, A_Wv))
    wo = A_Wo.reshape(H * E, D)
    any_spec = pl.BlockSpec(memory_space=pl.ANY)
    out = pl.pallas_call(
        _kernel,
        out_shape=jax.ShapeDtypeStruct((S_LEN, D), bf16),
        in_specs=[any_spec, pl.BlockSpec(memory_space=pltpu.VMEM)] + [any_spec] * 8,
        out_specs=any_spec,
        scratch_shapes=[
            pltpu.VMEM((S_LEN, D), bf16),
            pltpu.VMEM((RING, 4, PW, D), bf16),
            pltpu.VMEM((NP, 3, D // 2, PW), jnp.uint32),
            pltpu.VMEM((NP, PW // 2, D), jnp.uint32),
            pltpu.VMEM((D, D), bf16), pltpu.VMEM((D, D), bf16),
            pltpu.VMEM((D, F), bf16), pltpu.VMEM((F, D), bf16),
            pltpu.VMEM((XS_ROWS, D), f32), pltpu.VMEM((XS_ROWS, D), f32),
            pltpu.VMEM((XS_ROWS, D), f32),
            pltpu.VMEM((HB_ROWS, D), f32),
            pltpu.VMEM((2 * M_MEM, D), f32),
            pltpu.VMEM((XS_ROWS, D), bf16),
            pltpu.VMEM((3, PRE_ROWS, H * E), f32),
            pltpu.SemaphoreType.DMA((RING + 3,)),
            pltpu.SemaphoreType.DMA((2,)),
        ],
        compiler_params=pltpu.CompilerParams(vmem_limit_bytes=120 * 1024 * 1024),
        name="mem_mixer",
    )(x, mem0, wqt, wkt, wvt, wo, B_w1, B_w2, B_w3, B_w4)
    return out.reshape(1, S_LEN, D)
```

```python
import functools

import jax
import jax.numpy as jnp
import numpy as np
from jax import lax
import jax.experimental.pallas as pl
import jax.experimental.pallas.tpu as pltpu

f32 = jnp.float32
bf16 = jnp.bfloat16

S_LEN, D, H, E = 2048, 640, 32, 192
M_MEM, SEG = 8, 32
L = M_MEM + SEG
NSEG = S_LEN // SEG
NP = H // 2
PW = 2 * E
F = 1536
LAG = 3
RING = 4
PRE0, NPRE = LAG, 8
PRE_ROWS = L + NPRE * SEG
EPS = 1e-5
NEG = -1e30

NT = (((1,), (1,)), ((), ()))
NN = (((1,), (0,)), ((), ()))


def _dot(a, b, dims):
    return lax.dot_general(a, b, dims, preferred_element_type=f32)


def _ln(x):
    m = jnp.mean(x, axis=-1, keepdims=True)
    xc = x - m
    v = jnp.mean(xc * xc, axis=-1, keepdims=True)
    return xc * lax.rsqrt(v + EPS)


def _gelu(x):
    c = np.float32(np.sqrt(2.0 / np.pi))
    return 0.5 * x * (1.0 + jnp.tanh(c * (x + np.float32(0.044715) * (x * x * x))))


XS_DUMMY = S_LEN
XS_ROWS = S_LEN + SEG
HB_PAD = 8
HB_DUMMY = S_LEN + 2 * HB_PAD
HB_ROWS = HB_DUMMY + SEG + 2 * HB_PAD

ORDER_V80 = {
    'iter': [('k', 2), ('q', 2), ('s', 1), ('v', 2), ('pv', 0), ('out', -1)],
    (-2, 'pre'): ['b_pre'], (1, 'out'): ['b_mm1'], (4, 'k'): ['b_shift'], (5, 'end'): ['b_mm2'],
    (9, 'k'): ['x_ln'], (10, 'pv'): ['b_mm3:0'], (13, 'pv'): ['b_mm3:1'], (14, 'pre'): ['b_mm4:0'],
    (14, 's'): ['b_mm3:2', 'b_mm4:1'], (14, 'pv'): ['b_mm4:2'], (15, 'out'): ['b_fin'], (16, 'out'): ['a_fin'],
}
ORDER_V48 = {
    'iter': [('k', 2), ('q', 2), ('s', 1), ('pv', 0), ('v', 2), ('out', -1)],
    (-2, 'q'): ['b_pre'], (2, 'q'): ['b_mm1'], (3, 'q'): ['b_shift'], (6, 's'): ['b_mm2'],
    (9, 'end'): ['x_ln'], (11, 'pv'): ['b_mm3:0'], (11, 'end'): ['b_mm3:1'], (14, 's'): ['b_mm4:0'],
    (15, 'out'): ['b_mm3:2', 'b_mm4:1', 'b_mm4:2'], (15, 'end'): ['b_fin'], (16, 'out'): ['a_fin'],
}
ORDER_V40 = {
    'iter': [('k', 2), ('q', 2), ('v', 2), ('s', 1), ('pv', 0), ('out', -1)],
    (-2, 'end'): ['b_pre'], (6, 'v'): ['b_wait'], (7, 'k'): ['b_mm1'], (7, 'q'): ['b_shift'],
    (9, 'q'): ['b_mm2'], (12, 'k'): ['b_mm3:0'], (13, 'k'): ['b_mm3:1'], (13, 's'): ['b_mm3:2'],
    (14, 'pv'): ['b_mm4:0'], (15, 'pre'): ['b_mm4:1', 'b_mm4:2'], (15, 'end'): ['b_fin'], (16, 'out'): ['a_fin'],
}


def _kernel(x_hbm, mem0_ref, wq_hbm, wk_hbm, wv_hbm, wo_hbm, w1_hbm, w2_hbm, w3_hbm, w4_hbm,
            out_hbm,
            x_v, stg, wn, won, w1, w2, w3, w4, xs, lnx, ybuf, hbuf, mem, outs, pre, sems, osem):
    def pair_copies(p):
        r = pl.ds(pl.multiple_of(p * PW, PW), PW)
        slot = p % RING
        return [pltpu.make_async_copy(src.at[r], stg.at[slot, m], sems.at[slot])
                for m, src in enumerate((wk_hbm, wq_hbm, wv_hbm, wo_hbm))]

    n0 = (PRE0 + NPRE) * SEG
    x_cp0 = pltpu.make_async_copy(x_hbm.at[pl.ds(0, n0)], x_v.at[pl.ds(0, n0)], sems.at[RING])
    x_cp = pltpu.make_async_copy(x_hbm.at[pl.ds(n0, S_LEN - n0)], x_v.at[pl.ds(n0, S_LEN - n0)], sems.at[RING + 1])
    b_cps = [pltpu.make_async_copy(src, dst, sems.at[RING + 2])
             for src, dst in ((w1_hbm, w1), (w2_hbm, w2), (w3_hbm, w3), (w4_hbm, w4))]
    x_cp0.start()
    for p in range(RING - 1):
        for cp in pair_copies(p):
            cp.start()

    xs[pl.ds(XS_DUMMY, SEG), :] = jnp.zeros((SEG, D), f32)
    lnx[pl.ds(XS_DUMMY, SEG), :] = jnp.zeros((SEG, D), f32)
    ybuf[pl.ds(XS_DUMMY, SEG), :] = jnp.zeros((SEG, D), f32)
    hbuf[pl.ds(0, HB_PAD), :] = jnp.zeros((HB_PAD, D), f32)
    hbuf[pl.ds(HB_PAD + S_LEN, HB_ROWS - HB_PAD - S_LEN), :] = jnp.zeros((HB_ROWS - HB_PAD - S_LEN, D), f32)
    m0 = mem0_ref[...].astype(f32)
    mem[pl.ds(0, M_MEM), :] = m0
    mem[pl.ds(M_MEM, M_MEM), :] = m0
    x_cp0.wait()
    xf0 = x_v[pl.ds(0, n0), :].astype(f32)
    ln0 = _ln(xf0)
    xs[pl.ds(0, n0), :] = xf0
    lnx[pl.ds(0, n0), :] = ln0

    lane128 = lax.broadcasted_iota(jnp.int32, (L, 128), 1)
    lo64 = lane128 < 64
    l80 = lax.broadcasted_iota(jnp.int32, (L, 2 * L), 1)
    row = lax.broadcasted_iota(jnp.int32, (L, 2 * L), 0)
    ha = l80 < L
    key = jnp.where(ha, l80, l80 - L)
    allowed = (row < M_MEM) | (row >= key)
    scale = np.float32(E ** -0.5)
    z40 = jnp.zeros((L, 128), f32)
    lane32 = lax.broadcasted_iota(jnp.int32, (SEG, 128), 1)

    def seg_row(seg, dummy=XS_DUMMY):
        valid = jnp.logical_and(seg >= 0, seg < NSEG)
        return pl.multiple_of(jnp.where(valid, seg * SEG, dummy), 8)

    def blk(u):
        t0 = jnp.concatenate([u[:, 0:128], z40], axis=0)
        u1 = u[:, 128:256]
        t1 = jnp.concatenate([jnp.where(lo64, u1, 0.), jnp.where(lo64, 0., u1)], axis=0)
        t2 = jnp.concatenate([z40, u[:, 256:384]], axis=0)
        return jnp.concatenate([t0, t1, t2], axis=1).astype(bf16)

    def softmax_parts(s):
        xm = jnp.where(allowed, s * scale, np.float32(-1e9))
        m0_ = jnp.max(jnp.where(ha, xm, NEG), axis=1, keepdims=True)
        m1_ = jnp.max(jnp.where(ha, NEG, xm), axis=1, keepdims=True)
        pe = jnp.exp(xm - jnp.where(ha, m0_, m1_))
        i0 = 1.0 / jnp.sum(jnp.where(ha, pe, 0.), axis=1, keepdims=True)
        i1 = 1.0 / jnp.sum(jnp.where(ha, 0., pe), axis=1, keepdims=True)
        return pe, i0, i1

    def pv(parts, vb):
        pe, i0, i1 = parts
        o = _dot(pe, vb, NN)
        return jnp.concatenate([o[:, 0:128] * i0, o[:, 128:256] * jnp.where(lo64, i0, i1), o[:, 256:384] * i1],
                               axis=1)

    def make_stages(a_slots, ba_segs, bb_slots, pre_row=None, first_b=None):
        na = len(a_slots)
        st = {}
        a_rows = [seg_row(s) for s, _ in a_slots]
        ba_rows = [seg_row(s) for s in ba_segs]
        bb_rows = [seg_row(s) for s, _ in bb_slots]
        bah_rows = [seg_row(s, HB_DUMMY) + HB_PAD for s in ba_segs]
        bbh_rows = [seg_row(s, HB_DUMMY) for s, _ in bb_slots]
        fns = {}

        def stage(f):
            fns[f.__name__] = f
            return f

        if na:
            parts = []
            for l, ((_, mr), r) in enumerate(zip(a_slots, a_rows)):
                parts.append(mem[pl.ds(mr, M_MEM), :])
                if not (l == 0 and pre_row is not None):
                    parts.append(lnx[pl.ds(r, SEG), :])
            h = jnp.concatenate(parts, axis=0).astype(bf16 if na == 2 else f32)

        def proj(m, p):
            r = _dot(h, pltpu.bitcast(wn[p, m], bf16), NN)
            if pre_row is None:
                return [r[L * l:L * l + L] for l in range(na)]
            tok = pre[m, pl.ds(pre_row, SEG), pl.ds(PW * p, PW)]
            return [jnp.concatenate([r[0:M_MEM], tok], axis=0), r[M_MEM:M_MEM + L]]

        @stage
        def a_k(p):
            st['k', p] = [blk(k) for k in proj(0, p)]

        @stage
        def a_q(p):
            st['q', p] = proj(1, p)

        @stage
        def a_v(p):
            st['v', p] = [blk(v) for v in proj(2, p)]

        @stage
        def a_s(p):
            qs, ks = st.pop(('q', p)), st.pop(('k', p))
            st['p', p] = [softmax_parts(_dot(qs[l], ks[l], NT)) for l in range(na)]

        @stage
        def a_pv(p):
            ps, vs = st.pop(('p', p)), st.pop(('v', p))
            o = jnp.concatenate([pv(ps[l], vs[l]) for l in range(na)], axis=0)
            st['o', p] = o.astype(bf16) if na == 2 else o

        @stage
        def a_out(p):
            r = _dot(st.pop(('o', p)), pltpu.bitcast(won[p], bf16), NN)
            st['acc'] = r if 'acc' not in st else st['acc'] + r

        @stage
        def a_fin():
            acc = st.pop('acc')
            for l, ((_, mr), r) in enumerate(zip(a_slots, a_rows)):
                mem[pl.ds(mr, M_MEM), :] = acc[L * l:L * l + M_MEM]
                xs[pl.ds(r, SEG), :] = xs[pl.ds(r, SEG), :] + acc[L * l + M_MEM:L * l + L]

        @stage
        def x_ln():
            seg = a_slots[0][0] + NPRE
            src = pl.multiple_of(jnp.minimum(seg, NSEG - 1) * SEG, SEG)
            xf = x_v[pl.ds(src, SEG), :].astype(f32)
            r = seg_row(seg)
            xs[pl.ds(r, SEG), :] = xf
            lnx[pl.ds(r, SEG), :] = _ln(xf)

        @stage
        def b_wait():
            @pl.when(first_b)
            def _():
                for cp in b_cps:
                    cp.wait()

        @stage
        def b_pre():
            xa = jnp.concatenate([xs[pl.ds(r, SEG), :] for r in ba_rows], axis=0)
            y = _ln(xa)
            for l, r in enumerate(ba_rows):
                ybuf[pl.ds(r, SEG), :] = y[SEG * l:SEG * l + SEG]
            st['y2'] = _ln(y).astype(bf16)

        @stage
        def b_mm1():
            hh = _gelu(_dot(st.pop('y2'), w1[...], NN))
            for l, r in enumerate(bah_rows):
                hbuf[pl.ds(r, SEG), :] = hh[SEG * l:SEG * l + SEG]

        @stage
        def b_shift():
            parts = []
            for r in bbh_rows:
                win = hbuf[pl.ds(r, SEG + 2 * HB_PAD), :]

                def sh(d, c):
                    return win[HB_PAD + d:HB_PAD + d + SEG, 128 * c:128 * c + 128]
                parts.append(jnp.concatenate([
                    sh(-1, 0),
                    jnp.where(lane32 < 32, sh(-1, 1), sh(1, 1)),
                    jnp.where(lane32 < 64, sh(1, 2), sh(-2, 2)),
                    jnp.where(lane32 < 96, sh(-2, 3), sh(2, 3)),
                    sh(2, 4)], axis=1))
            st['hsft'] = jnp.concatenate(parts, axis=0).astype(bf16)

        @stage
        def b_mm2():
            hs = _dot(st.pop('hsft'), w2[...], NN)
            y = jnp.concatenate([ybuf[pl.ds(r, SEG), :] for r in bb_rows], axis=0)
            x1 = y + hs
            xa = jnp.concatenate([xs[pl.ds(r, SEG), :] for r in bb_rows], axis=0)
            st['res'] = xa + x1
            st['z'] = _ln(x1).astype(bf16)

        @stage
        def b_mm3(c):
            st['g', c] = _gelu(_dot(st['z'], w3[:, pl.ds(512 * c, 512)], NN)).astype(bf16)

        @stage
        def b_mm4(c):
            st['res'] = st['res'] + _dot(st.pop(('g', c)), w4[pl.ds(512 * c, 512), :], NN)

        @stage
        def b_fin():
            o = st.pop('res')
            for l, ((_, final), r) in enumerate(zip(bb_slots, bb_rows)):
                ol = o[SEG * l:SEG * l + SEG]
                if final:
                    outs[pl.ds(r, SEG), :] = ol.astype(bf16)
                else:
                    xs[pl.ds(r, SEG), :] = ol
                    lnx[pl.ds(r, SEG), :] = _ln(ol)

        def run(name):
            if ':' in name:
                n, a = name.split(':')
                fns[n](int(a))
            else:
                fns[name]()
        return run

    def run_order(run, order):
        offs = [o for _, o in order['iter']]
        for i in range(-max(offs), NP - min(offs)):
            sched = list(order.get((i, 'pre'), []))
            for name, o in order['iter']:
                if 0 <= i + o < NP:
                    sched.append('a_%s:%d' % (name, i + o))
                    sched += order.get((i, name), [])
            sched += order.get((i, 'end'), [])
            for s in sched:
                run(s)

    def b_slots(t):
        return ([t - 1, t - LAG - 1], [(t - 2, False), (t - LAG - 2, True)])

    h0 = jnp.concatenate([m0, ln0[0:SEG], ln0[PRE0 * SEG:n0]], axis=0)

    def attend0(p):
        c = pl.ds(pl.multiple_of(p * PW, PW), PW)
        st = {}

        def a_s():
            st['p'] = softmax_parts(_dot(pre[1, pl.ds(0, L), c], blk(pre[0, pl.ds(0, L), c]), NT))

        def a_pv():
            st['o'] = pv(st['p'], blk(pre[2, pl.ds(0, L), c]))

        def a_out(acc):
            return acc + _dot(st['o'], pltpu.bitcast(won[p], bf16), NN)
        return a_s, a_pv, a_out

    for m in range(3):
        pre[m, pl.ds(0, L), pl.ds(0, PW)] = jnp.zeros((L, PW), f32)

    def first(p, acc):
        @pl.when(p + RING - 1 < NP)
        def _():
            for cp in pair_copies(jnp.minimum(p + RING - 1, NP - 1)):
                cp.start()

        @pl.when(p + RING - 1 == NP)
        def _():
            for cp in b_cps:
                cp.start()
            x_cp.start()
        for cp in pair_copies(p):
            cp.wait()
        slot = p % RING
        c = pl.ds(pl.multiple_of(p * PW, PW), PW)
        a_s, a_pv, a_out = attend0(jnp.maximum(p - 1, 0))

        def proj0(m):
            w = stg[slot, m]
            wn[p, m] = pltpu.bitcast(jnp.transpose(w), jnp.uint32)
            return _dot(h0, w, NT)
        won[p] = pltpu.bitcast(stg[slot, 3], jnp.uint32)
        k = proj0(0)
        a_s()
        pre_q = proj0(1)
        a_pv()
        pre[0, :, c] = k
        pre[1, :, c] = pre_q
        v = proj0(2)
        acc = a_out(acc)
        pre[2, :, c] = v
        return acc
    acc0 = lax.fori_loop(0, NP, first, jnp.zeros((L, D), f32))
    a_s, a_pv, a_out = attend0(NP - 1)
    a_s()
    a_pv()
    acc0 = a_out(acc0)
    mem[pl.ds(0, M_MEM), :] = acc0[0:M_MEM]
    xs[pl.ds(0, SEG), :] = xs[pl.ds(0, SEG), :] + acc0[M_MEM:L]

    def step(t, carry):
        pre_on = jnp.logical_and(t >= PRE0, t < PRE0 + NPRE)
        full = jnp.logical_and(t >= PRE0 + NPRE, t < NSEG)
        single = jnp.logical_or(t < LAG, t >= NSEG)

        @pl.when(t == LAG)
        def _():
            x_cp.wait()

        @pl.when(full)
        def _():
            ba, bb = b_slots(t)
            run_order(make_stages([(t, 0), (t - LAG, M_MEM)], ba, bb), ORDER_V80)

        @pl.when(pre_on)
        def _():
            ba, bb = b_slots(t)
            pr = pl.multiple_of(L + (jnp.clip(t, PRE0, PRE0 + NPRE - 1) - PRE0) * SEG, 8)
            run_order(make_stages([(t, 0), (t - LAG, M_MEM)], ba, bb, pre_row=pr), ORDER_V48)

        @pl.when(single)
        def _():
            ba, bb = b_slots(t)
            early = t < LAG
            seg = jnp.where(early, t, t - LAG)
            mr = pl.multiple_of(jnp.where(early, 0, M_MEM), M_MEM)
            run_order(make_stages([(seg, mr)], ba, bb, first_b=(t == 1)), ORDER_V40)
        return carry
    lax.fori_loop(1, NSEG + LAG, step, 0)

    n_done = NSEG - 2
    cp_a = pltpu.make_async_copy(outs.at[pl.ds(0, n_done * SEG)], out_hbm.at[pl.ds(0, n_done * SEG)], osem.at[0])
    cp_a.start()
    run = make_stages([], [NSEG - 1], [(NSEG - 2, True), (NSEG - 1, True)])
    for s in ['b_pre', 'b_mm1', 'b_shift', 'b_mm2', 'b_mm3:0', 'b_mm3:1', 'b_mm3:2', 'b_mm4:0', 'b_mm4:1', 'b_mm4:2',
              'b_fin']:
        run(s)
    cp_b = pltpu.make_async_copy(outs.at[pl.ds(n_done * SEG, 2 * SEG)], out_hbm.at[pl.ds(n_done * SEG, 2 * SEG)],
                                 osem.at[1])
    cp_b.start()
    cp_a.wait()
    cp_b.wait()


@functools.partial(jax.jit, static_argnames=("A_seg_len",))
def pallas_interleave_layers__memory_aug_recurrent_mem_tr__mixer_s_mlp__prompt_kernel(
        A_x, A_mem0, A_Wq, A_Wk, A_Wv, A_Wo, A_seg_len, B_x, B_w1, B_w2, B_w3, B_w4):
    del B_x
    assert A_seg_len == SEG and A_x.shape == (1, S_LEN, D) and A_Wq.shape == (D, H, E)
    x = A_x.reshape(S_LEN, D)
    mem0 = A_mem0.reshape(M_MEM, D)
    wqt, wkt, wvt = (jnp.transpose(w, (1, 2, 0)).reshape(H * E, D) for w in (A_Wq, A_Wk, A_Wv))
    wo = A_Wo.reshape(H * E, D)
    any_spec = pl.BlockSpec(memory_space=pl.ANY)
    out = pl.pallas_call(
        _kernel,
        out_shape=jax.ShapeDtypeStruct((S_LEN, D), bf16),
        in_specs=[any_spec, pl.BlockSpec(memory_space=pltpu.VMEM)] + [any_spec] * 8,
        out_specs=any_spec,
        scratch_shapes=[
            pltpu.VMEM((S_LEN, D), bf16),
            pltpu.VMEM((RING, 4, PW, D), bf16),
            pltpu.VMEM((NP, 3, D // 2, PW), jnp.uint32),
            pltpu.VMEM((NP, PW // 2, D), jnp.uint32),
            pltpu.VMEM((D, D), bf16), pltpu.VMEM((D, D), bf16),
            pltpu.VMEM((D, F), bf16), pltpu.VMEM((F, D), bf16),
            pltpu.VMEM((XS_ROWS, D), f32), pltpu.VMEM((XS_ROWS, D), f32),
            pltpu.VMEM((XS_ROWS, D), f32),
            pltpu.VMEM((HB_ROWS, D), f32),
            pltpu.VMEM((2 * M_MEM, D), f32),
            pltpu.VMEM((XS_ROWS, D), bf16),
            pltpu.VMEM((3, PRE_ROWS, H * E), f32),
            pltpu.SemaphoreType.DMA((RING + 3,)),
            pltpu.SemaphoreType.DMA((2,)),
        ],
        compiler_params=pltpu.CompilerParams(vmem_limit_bytes=120 * 1024 * 1024),
        name="mem_mixer",
    )(x, mem0, wqt, wkt, wvt, wo, B_w1, B_w2, B_w3, B_w4)
    return out.reshape(1, S_LEN, D)
```

```python
import functools

import jax
import jax.numpy as jnp
import numpy as np
from jax import lax
import jax.experimental.pallas as pl
import jax.experimental.pallas.tpu as pltpu

f32 = jnp.float32
bf16 = jnp.bfloat16

S_LEN, D, H, E = 2048, 640, 32, 192
M_MEM, SEG = 8, 32
L = M_MEM + SEG
NSEG = S_LEN // SEG
NP = H // 2
PW = 2 * E
F = 1536
LAG = 3
RING = 4
PRE0, NPRE = LAG, 8
PRE_ROWS = L + NPRE * SEG
EPS = 1e-5
NEG = -1e30

NT = (((1,), (1,)), ((), ()))
NN = (((1,), (0,)), ((), ()))


def _dot(a, b, dims):
    return lax.dot_general(a, b, dims, preferred_element_type=f32)


def _ln(x):
    m = jnp.mean(x, axis=-1, keepdims=True)
    xc = x - m
    v = jnp.mean(xc * xc, axis=-1, keepdims=True)
    return xc * lax.rsqrt(v + EPS)


def _gelu(x):
    c = np.float32(np.sqrt(2.0 / np.pi))
    return 0.5 * x * (1.0 + jnp.tanh(c * (x + np.float32(0.044715) * (x * x * x))))


XS_DUMMY = S_LEN
XS_ROWS = S_LEN + SEG
HB_PAD = 8
HB_DUMMY = S_LEN + 2 * HB_PAD
HB_ROWS = HB_DUMMY + SEG + 2 * HB_PAD

ORDER_V0 = ['wk', 'wq', 'wv', 'wo', 's', 'to', 'tk', 'k', 'pv', 'tq', 'q', 'out', 'tv', 'v']
ORDER_V80 = {
    'iter': [('k', 2), ('q', 2), ('s', 1), ('v', 2), ('pv', 0), ('out', -1)],
    (-2, 'pre'): ['b_pre'], (1, 'out'): ['b_mm1'], (4, 'k'): ['b_shift'], (5, 'end'): ['b_mm2'],
    (9, 'k'): ['x_ln'], (10, 'pv'): ['b_mm3:0'], (13, 'pv'): ['b_mm3:1'], (14, 'pre'): ['b_mm4:0'],
    (14, 's'): ['b_mm3:2', 'b_mm4:1'], (14, 'pv'): ['b_mm4:2'], (15, 'out'): ['b_fin'], (16, 'out'): ['a_fin'],
}
ORDER_V48 = {
    'iter': [('k', 2), ('q', 2), ('s', 1), ('pv', 0), ('v', 2), ('out', -1)],
    (-2, 'q'): ['b_pre'], (2, 'q'): ['b_mm1'], (3, 'q'): ['b_shift'], (6, 's'): ['b_mm2'],
    (9, 'end'): ['x_ln'], (11, 'pv'): ['b_mm3:0'], (11, 'end'): ['b_mm3:1'], (14, 's'): ['b_mm4:0'],
    (15, 'out'): ['b_mm3:2', 'b_mm4:1', 'b_mm4:2'], (15, 'end'): ['b_fin'], (16, 'out'): ['a_fin'],
}
ORDER_V40 = {
    'iter': [('k', 2), ('q', 2), ('v', 2), ('s', 1), ('pv', 0), ('out', -1)],
    (-2, 'end'): ['b_pre'], (6, 'v'): ['b_wait'], (7, 'k'): ['b_mm1'], (7, 'q'): ['b_shift'],
    (9, 'q'): ['b_mm2'], (12, 'k'): ['b_mm3:0'], (13, 'k'): ['b_mm3:1'], (13, 's'): ['b_mm3:2'],
    (14, 'pv'): ['b_mm4:0'], (15, 'pre'): ['b_mm4:1', 'b_mm4:2'], (15, 'end'): ['b_fin'], (16, 'out'): ['a_fin'],
}


def _kernel(x_hbm, mem0_ref, wq_hbm, wk_hbm, wv_hbm, wo_hbm, w1_hbm, w2_hbm, w3_hbm, w4_hbm,
            out_hbm,
            x_v, stg, wn, won, w1, w2, w3, w4, xs, lnx, ybuf, hbuf, mem, outs, pre, sems, osem):
    def pair_copies(p):
        r = pl.ds(pl.multiple_of(p * PW, PW), PW)
        slot = p % RING
        return [pltpu.make_async_copy(src.at[r], stg.at[slot, m], sems.at[slot * 4 + m])
                for m, src in enumerate((wk_hbm, wq_hbm, wv_hbm, wo_hbm))]

    n0 = (PRE0 + NPRE) * SEG
    x_cp0 = pltpu.make_async_copy(x_hbm.at[pl.ds(0, n0)], x_v.at[pl.ds(0, n0)], sems.at[4 * RING])
    x_cp = pltpu.make_async_copy(x_hbm.at[pl.ds(n0, S_LEN - n0)], x_v.at[pl.ds(n0, S_LEN - n0)], sems.at[4 * RING + 1])
    b_cps = [pltpu.make_async_copy(src, dst, sems.at[4 * RING + 2])
             for src, dst in ((w1_hbm, w1), (w2_hbm, w2), (w3_hbm, w3), (w4_hbm, w4))]
    x_cp0.start()
    for p in range(RING):
        for cp in pair_copies(p):
            cp.start()

    xs[pl.ds(XS_DUMMY, SEG), :] = jnp.zeros((SEG, D), f32)
    lnx[pl.ds(XS_DUMMY, SEG), :] = jnp.zeros((SEG, D), f32)
    ybuf[pl.ds(XS_DUMMY, SEG), :] = jnp.zeros((SEG, D), f32)
    hbuf[pl.ds(0, HB_PAD), :] = jnp.zeros((HB_PAD, D), f32)
    hbuf[pl.ds(HB_PAD + S_LEN, HB_ROWS - HB_PAD - S_LEN), :] = jnp.zeros((HB_ROWS - HB_PAD - S_LEN, D), f32)
    m0 = mem0_ref[...].astype(f32)
    mem[pl.ds(0, M_MEM), :] = m0
    mem[pl.ds(M_MEM, M_MEM), :] = m0
    x_cp0.wait()
    xf0 = x_v[pl.ds(0, n0), :].astype(f32)
    ln0 = _ln(xf0)
    xs[pl.ds(0, n0), :] = xf0
    lnx[pl.ds(0, n0), :] = ln0

    lane128 = lax.broadcasted_iota(jnp.int32, (L, 128), 1)
    lo64 = lane128 < 64
    l80 = lax.broadcasted_iota(jnp.int32, (L, 2 * L), 1)
    row = lax.broadcasted_iota(jnp.int32, (L, 2 * L), 0)
    ha = l80 < L
    key = jnp.where(ha, l80, l80 - L)
    allowed = (row < M_MEM) | (row >= key)
    scale = np.float32(E ** -0.5)
    z40 = jnp.zeros((L, 128), f32)
    lane32 = lax.broadcasted_iota(jnp.int32, (SEG, 128), 1)

    def seg_row(seg, dummy=XS_DUMMY):
        valid = jnp.logical_and(seg >= 0, seg < NSEG)
        return pl.multiple_of(jnp.where(valid, seg * SEG, dummy), 8)

    def blk(u):
        t0 = jnp.concatenate([u[:, 0:128], z40], axis=0)
        u1 = u[:, 128:256]
        t1 = jnp.concatenate([jnp.where(lo64, u1, 0.), jnp.where(lo64, 0., u1)], axis=0)
        t2 = jnp.concatenate([z40, u[:, 256:384]], axis=0)
        return jnp.concatenate([t0, t1, t2], axis=1).astype(bf16)

    def softmax_parts(s):
        xm = jnp.where(allowed, s * scale, np.float32(-1e9))
        m0_ = jnp.max(jnp.where(ha, xm, NEG), axis=1, keepdims=True)
        m1_ = jnp.max(jnp.where(ha, NEG, xm), axis=1, keepdims=True)
        pe = jnp.exp(xm - jnp.where(ha, m0_, m1_))
        i0 = 1.0 / jnp.sum(jnp.where(ha, pe, 0.), axis=1, keepdims=True)
        i1 = 1.0 / jnp.sum(jnp.where(ha, 0., pe), axis=1, keepdims=True)
        return pe, i0, i1

    def pv(parts, vb):
        pe, i0, i1 = parts
        o = _dot(pe, vb, NN)
        return jnp.concatenate([o[:, 0:128] * i0, o[:, 128:256] * jnp.where(lo64, i0, i1), o[:, 256:384] * i1],
                               axis=1)

    def make_stages(a_slots, ba_segs, bb_slots, pre_row=None, first_b=None):
        na = len(a_slots)
        st = {}
        a_rows = [seg_row(s) for s, _ in a_slots]
        ba_rows = [seg_row(s) for s in ba_segs]
        bb_rows = [seg_row(s) for s, _ in bb_slots]
        bah_rows = [seg_row(s, HB_DUMMY) + HB_PAD for s in ba_segs]
        bbh_rows = [seg_row(s, HB_DUMMY) for s, _ in bb_slots]
        fns = {}

        def stage(f):
            fns[f.__name__] = f
            return f

        if na:
            parts = []
            for l, ((_, mr), r) in enumerate(zip(a_slots, a_rows)):
                parts.append(mem[pl.ds(mr, M_MEM), :])
                if not (l == 0 and pre_row is not None):
                    parts.append(lnx[pl.ds(r, SEG), :])
            h = jnp.concatenate(parts, axis=0).astype(bf16 if na == 2 else f32)

        def proj(m, p):
            r = _dot(h, pltpu.bitcast(wn[p, m], bf16), NN)
            if pre_row is None:
                return [r[L * l:L * l + L] for l in range(na)]
            tok = pre[m, pl.ds(pre_row, SEG), pl.ds(PW * p, PW)]
            return [jnp.concatenate([r[0:M_MEM], tok], axis=0), r[M_MEM:M_MEM + L]]

        @stage
        def a_k(p):
            st['k', p] = [blk(k) for k in proj(0, p)]

        @stage
        def a_q(p):
            st['q', p] = proj(1, p)

        @stage
        def a_v(p):
            st['v', p] = [blk(v) for v in proj(2, p)]

        @stage
        def a_s(p):
            qs, ks = st.pop(('q', p)), st.pop(('k', p))
            st['p', p] = [softmax_parts(_dot(qs[l], ks[l], NT)) for l in range(na)]

        @stage
        def a_pv(p):
            ps, vs = st.pop(('p', p)), st.pop(('v', p))
            o = jnp.concatenate([pv(ps[l], vs[l]) for l in range(na)], axis=0)
            st['o', p] = o.astype(bf16) if na == 2 else o

        @stage
        def a_out(p):
            r = _dot(st.pop(('o', p)), pltpu.bitcast(won[p], bf16), NN)
            st['acc'] = r if 'acc' not in st else st['acc'] + r

        @stage
        def a_fin():
            acc = st.pop('acc')
            for l, ((_, mr), r) in enumerate(zip(a_slots, a_rows)):
                mem[pl.ds(mr, M_MEM), :] = acc[L * l:L * l + M_MEM]
                xs[pl.ds(r, SEG), :] = xs[pl.ds(r, SEG), :] + acc[L * l + M_MEM:L * l + L]

        @stage
        def x_ln():
            seg = a_slots[0][0] + NPRE
            src = pl.multiple_of(jnp.minimum(seg, NSEG - 1) * SEG, SEG)
            xf = x_v[pl.ds(src, SEG), :].astype(f32)
            r = seg_row(seg)
            xs[pl.ds(r, SEG), :] = xf
            lnx[pl.ds(r, SEG), :] = _ln(xf)

        @stage
        def b_wait():
            @pl.when(first_b)
            def _():
                for cp in b_cps:
                    cp.wait()

        @stage
        def b_pre():
            xa = jnp.concatenate([xs[pl.ds(r, SEG), :] for r in ba_rows], axis=0)
            y = _ln(xa)
            for l, r in enumerate(ba_rows):
                ybuf[pl.ds(r, SEG), :] = y[SEG * l:SEG * l + SEG]
            st['y2'] = _ln(y).astype(bf16)

        @stage
        def b_mm1():
            hh = _gelu(_dot(st.pop('y2'), w1[...], NN))
            for l, r in enumerate(bah_rows):
                hbuf[pl.ds(r, SEG), :] = hh[SEG * l:SEG * l + SEG]

        @stage
        def b_shift():
            parts = []
            for r in bbh_rows:
                win = hbuf[pl.ds(r, SEG + 2 * HB_PAD), :]

                def sh(d, c):
                    return win[HB_PAD + d:HB_PAD + d + SEG, 128 * c:128 * c + 128]
                parts.append(jnp.concatenate([
                    sh(-1, 0),
                    jnp.where(lane32 < 32, sh(-1, 1), sh(1, 1)),
                    jnp.where(lane32 < 64, sh(1, 2), sh(-2, 2)),
                    jnp.where(lane32 < 96, sh(-2, 3), sh(2, 3)),
                    sh(2, 4)], axis=1))
            st['hsft'] = jnp.concatenate(parts, axis=0).astype(bf16)

        @stage
        def b_mm2():
            hs = _dot(st.pop('hsft'), w2[...], NN)
            y = jnp.concatenate([ybuf[pl.ds(r, SEG), :] for r in bb_rows], axis=0)
            x1 = y + hs
            xa = jnp.concatenate([xs[pl.ds(r, SEG), :] for r in bb_rows], axis=0)
            st['res'] = xa + x1
            st['z'] = _ln(x1).astype(bf16)

        @stage
        def b_mm3(c):
            st['g', c] = _gelu(_dot(st['z'], w3[:, pl.ds(512 * c, 512)], NN)).astype(bf16)

        @stage
        def b_mm4(c):
            st['res'] = st['res'] + _dot(st.pop(('g', c)), w4[pl.ds(512 * c, 512), :], NN)

        @stage
        def b_fin():
            o = st.pop('res')
            for l, ((_, final), r) in enumerate(zip(bb_slots, bb_rows)):
                ol = o[SEG * l:SEG * l + SEG]
                if final:
                    outs[pl.ds(r, SEG), :] = ol.astype(bf16)
                else:
                    xs[pl.ds(r, SEG), :] = ol
                    lnx[pl.ds(r, SEG), :] = _ln(ol)

        def run(name):
            if ':' in name:
                n, a = name.split(':')
                fns[n](int(a))
            else:
                fns[name]()
        return run

    def run_order(run, order):
        offs = [o for _, o in order['iter']]
        for i in range(-max(offs), NP - min(offs)):
            sched = list(order.get((i, 'pre'), []))
            for name, o in order['iter']:
                if 0 <= i + o < NP:
                    sched.append('a_%s:%d' % (name, i + o))
                    sched += order.get((i, name), [])
            sched += order.get((i, 'end'), [])
            for s in sched:
                run(s)

    def b_slots(t):
        return ([t - 1, t - LAG - 1], [(t - 2, False), (t - LAG - 2, True)])

    h0 = jnp.concatenate([m0, ln0[0:SEG], ln0[PRE0 * SEG:n0]], axis=0)

    def attend0(p):
        c = pl.ds(pl.multiple_of(p * PW, PW), PW)
        st = {}
        k0, q0, v0 = (pre[m, pl.ds(0, L), c] for m in range(3))

        def a_s():
            st['p'] = softmax_parts(_dot(q0, blk(k0), NT))

        def a_pv():
            st['o'] = pv(st['p'], blk(v0))

        def a_out(acc):
            return acc + _dot(st['o'], pltpu.bitcast(won[p], bf16), NN)
        return a_s, a_pv, a_out

    for m in range(3):
        pre[m, pl.ds(0, L), pl.ds(0, PW)] = jnp.zeros((L, PW), f32)

    def first(p, acc):
        cps = pair_copies(p)
        slot = p % RING
        c = pl.ds(pl.multiple_of(p * PW, PW), PW)
        a_s, a_pv, a_out = attend0(jnp.maximum(p - 1, 0))

        st = {'acc': acc}

        def proj0(m):
            pre[m, :, c] = _dot(h0, stg[slot, m], NT)

        def retile(m):
            w = stg[slot, m]
            if m < 3:
                wn[p, m] = pltpu.bitcast(jnp.transpose(w), jnp.uint32)
            else:
                won[p] = pltpu.bitcast(w, jnp.uint32)

        def out0():
            st['acc'] = a_out(st['acc'])
        ops = {'k': lambda: proj0(0), 'q': lambda: proj0(1), 'v': lambda: proj0(2),
               'tk': lambda: retile(0), 'tq': lambda: retile(1), 'tv': lambda: retile(2), 'to': lambda: retile(3),
               'wk': cps[0].wait, 'wq': cps[1].wait, 'wv': cps[2].wait, 'wo': cps[3].wait,
               's': a_s, 'pv': a_pv, 'out': out0}
        for name in ORDER_V0:
            ops[name]()
        acc = st['acc']

        @pl.when(p + RING < NP)
        def _():
            for cp in pair_copies(jnp.minimum(p + RING, NP - 1)):
                cp.start()

        @pl.when(p + RING == NP)
        def _():
            for cp in b_cps:
                cp.start()
            x_cp.start()
        return acc
    acc0 = lax.fori_loop(0, NP, first, jnp.zeros((L, D), f32))
    a_s, a_pv, a_out = attend0(NP - 1)
    a_s()
    a_pv()
    acc0 = a_out(acc0)
    mem[pl.ds(0, M_MEM), :] = acc0[0:M_MEM]
    xs[pl.ds(0, SEG), :] = xs[pl.ds(0, SEG), :] + acc0[M_MEM:L]

    def step(t, carry):
        pre_on = jnp.logical_and(t >= PRE0, t < PRE0 + NPRE)
        full = jnp.logical_and(t >= PRE0 + NPRE, t < NSEG)
        single = jnp.logical_or(t < LAG, t >= NSEG)

        @pl.when(t == LAG)
        def _():
            x_cp.wait()

        @pl.when(full)
        def _():
            ba, bb = b_slots(t)
            run_order(make_stages([(t, 0), (t - LAG, M_MEM)], ba, bb), ORDER_V80)

        @pl.when(pre_on)
        def _():
            ba, bb = b_slots(t)
            pr = pl.multiple_of(L + (jnp.clip(t, PRE0, PRE0 + NPRE - 1) - PRE0) * SEG, 8)
            run_order(make_stages([(t, 0), (t - LAG, M_MEM)], ba, bb, pre_row=pr), ORDER_V48)

        @pl.when(single)
        def _():
            ba, bb = b_slots(t)
            early = t < LAG
            seg = jnp.where(early, t, t - LAG)
            mr = pl.multiple_of(jnp.where(early, 0, M_MEM), M_MEM)
            run_order(make_stages([(seg, mr)], ba, bb, first_b=(t == 1)), ORDER_V40)
        return carry
    lax.fori_loop(1, NSEG + LAG, step, 0)

    n_done = NSEG - 2
    cp_a = pltpu.make_async_copy(outs.at[pl.ds(0, n_done * SEG)], out_hbm.at[pl.ds(0, n_done * SEG)], osem.at[0])
    cp_a.start()
    run = make_stages([], [NSEG - 1], [(NSEG - 2, True), (NSEG - 1, True)])
    for s in ['b_pre', 'b_mm1', 'b_shift', 'b_mm2', 'b_mm3:0', 'b_mm3:1', 'b_mm3:2', 'b_mm4:0', 'b_mm4:1', 'b_mm4:2',
              'b_fin']:
        run(s)
    cp_b = pltpu.make_async_copy(outs.at[pl.ds(n_done * SEG, 2 * SEG)], out_hbm.at[pl.ds(n_done * SEG, 2 * SEG)],
                                 osem.at[1])
    cp_b.start()
    cp_a.wait()
    cp_b.wait()


@functools.partial(jax.jit, static_argnames=("A_seg_len",))
def pallas_interleave_layers__memory_aug_recurrent_mem_tr__mixer_s_mlp__prompt_kernel(
        A_x, A_mem0, A_Wq, A_Wk, A_Wv, A_Wo, A_seg_len, B_x, B_w1, B_w2, B_w3, B_w4):
    del B_x
    assert A_seg_len == SEG and A_x.shape == (1, S_LEN, D) and A_Wq.shape == (D, H, E)
    x = A_x.reshape(S_LEN, D)
    mem0 = A_mem0.reshape(M_MEM, D)
    wqt, wkt, wvt = (jnp.transpose(w, (1, 2, 0)).reshape(H * E, D) for w in (A_Wq, A_Wk, A_Wv))
    wo = A_Wo.reshape(H * E, D)
    any_spec = pl.BlockSpec(memory_space=pl.ANY)
    out = pl.pallas_call(
        _kernel,
        out_shape=jax.ShapeDtypeStruct((S_LEN, D), bf16),
        in_specs=[any_spec, pl.BlockSpec(memory_space=pltpu.VMEM)] + [any_spec] * 8,
        out_specs=any_spec,
        scratch_shapes=[
            pltpu.VMEM((S_LEN, D), bf16),
            pltpu.VMEM((RING, 4, PW, D), bf16),
            pltpu.VMEM((NP, 3, D // 2, PW), jnp.uint32),
            pltpu.VMEM((NP, PW // 2, D), jnp.uint32),
            pltpu.VMEM((D, D), bf16), pltpu.VMEM((D, D), bf16),
            pltpu.VMEM((D, F), bf16), pltpu.VMEM((F, D), bf16),
            pltpu.VMEM((XS_ROWS, D), f32), pltpu.VMEM((XS_ROWS, D), f32),
            pltpu.VMEM((XS_ROWS, D), f32),
            pltpu.VMEM((HB_ROWS, D), f32),
            pltpu.VMEM((2 * M_MEM, D), f32),
            pltpu.VMEM((XS_ROWS, D), bf16),
            pltpu.VMEM((3, PRE_ROWS, H * E), f32),
            pltpu.SemaphoreType.DMA((4 * RING + 3,)),
            pltpu.SemaphoreType.DMA((2,)),
        ],
        compiler_params=pltpu.CompilerParams(vmem_limit_bytes=120 * 1024 * 1024),
        name="mem_mixer",
    )(x, mem0, wqt, wkt, wvt, wo, B_w1, B_w2, B_w3, B_w4)
    return out.reshape(1, S_LEN, D)
```

```python
import functools

import jax
import jax.numpy as jnp
import numpy as np
from jax import lax
import jax.experimental.pallas as pl
import jax.experimental.pallas.tpu as pltpu

f32 = jnp.float32
bf16 = jnp.bfloat16

S_LEN, D, H, E = 2048, 640, 32, 192
M_MEM, SEG = 8, 32
L = M_MEM + SEG
NSEG = S_LEN // SEG
NP = H // 2
PW = 2 * E
F = 1536
LAG = 3
RING = 4
PRE0, NPRE = LAG, 8
PRE_ROWS = L + NPRE * SEG
EPS = 1e-5
NEG = -1e30

NT = (((1,), (1,)), ((), ()))
NN = (((1,), (0,)), ((), ()))


def _dot(a, b, dims):
    return lax.dot_general(a, b, dims, preferred_element_type=f32)


def _ln(x):
    m = jnp.mean(x, axis=-1, keepdims=True)
    xc = x - m
    v = jnp.mean(xc * xc, axis=-1, keepdims=True)
    return xc * lax.rsqrt(v + EPS)


def _gelu(x):
    c = np.float32(np.sqrt(2.0 / np.pi))
    return 0.5 * x * (1.0 + jnp.tanh(c * (x + np.float32(0.044715) * (x * x * x))))


XS_DUMMY = S_LEN
XS_ROWS = S_LEN + SEG
HB_PAD = 8
HB_DUMMY = S_LEN + 2 * HB_PAD
HB_ROWS = HB_DUMMY + SEG + 2 * HB_PAD

ORDER_V0 = ['wk', 'wq', 'wv', 'wo', 's', 'to', 'tk', 'k', 'pv', 'tq', 'q', 'out', 'tv', 'v']
ORDER_V80 = {
    'iter': [('k', 2), ('q', 2), ('s', 1), ('v', 2), ('pv', 0), ('out', -1)],
    (-2, 'pre'): ['b_pre'], (1, 'out'): ['b_mm1'], (4, 'k'): ['b_shift'], (5, 'end'): ['b_mm2'],
    (9, 'k'): ['x_ln'], (10, 'pv'): ['b_mm3:0'], (13, 'pv'): ['b_mm3:1'], (14, 'pre'): ['b_mm4:0'],
    (14, 's'): ['b_mm3:2', 'b_mm4:1'], (14, 'pv'): ['b_mm4:2'], (15, 'out'): ['b_fin'], (16, 'out'): ['a_fin'],
}
ORDER_V48 = {
    'iter': [('k', 2), ('q', 2), ('s', 1), ('pv', 0), ('v', 2), ('out', -1)],
    (-2, 'q'): ['b_pre'], (2, 'q'): ['b_mm1'], (3, 'q'): ['b_shift'], (6, 's'): ['b_mm2'],
    (9, 'end'): ['x_ln'], (11, 'pv'): ['b_mm3:0'], (11, 'end'): ['b_mm3:1'], (14, 's'): ['b_mm4:0'],
    (15, 'out'): ['b_mm3:2', 'b_mm4:1', 'b_mm4:2'], (15, 'end'): ['b_fin'], (16, 'out'): ['a_fin'],
}
ORDER_V40 = {
    'iter': [('k', 2), ('q', 2), ('v', 2), ('s', 1), ('pv', 0), ('out', -1)],
    (-2, 'end'): ['b_pre'], (6, 'v'): ['b_wait'], (7, 'k'): ['b_mm1'], (7, 'q'): ['b_shift'],
    (9, 'q'): ['b_mm2'], (12, 'k'): ['b_mm3:0'], (13, 'k'): ['b_mm3:1'], (13, 's'): ['b_mm3:2'],
    (14, 'pv'): ['b_mm4:0'], (15, 'pre'): ['b_mm4:1', 'b_mm4:2'], (15, 'end'): ['b_fin'], (16, 'out'): ['a_fin'],
}


def _kernel(x_hbm, mem0_ref, wq_hbm, wk_hbm, wv_hbm, wo_hbm, w1_hbm, w2_hbm, w3_hbm, w4_hbm,
            out_hbm,
            x_v, stg, wn, won, w1, w2, w3, w4, xs, lnx, ybuf, hbuf, mem, outs, pre, sems, osem):
    def pair_copies(p):
        r = pl.ds(pl.multiple_of(p * PW, PW), PW)
        slot = p % RING
        return [pltpu.make_async_copy(src.at[r], stg.at[slot, m], sems.at[slot * 4 + m])
                for m, src in enumerate((wk_hbm, wq_hbm, wv_hbm, wo_hbm))]

    n0 = (PRE0 + NPRE) * SEG
    x_cp0 = pltpu.make_async_copy(x_hbm.at[pl.ds(0, n0)], x_v.at[pl.ds(0, n0)], sems.at[4 * RING])
    x_cp = pltpu.make_async_copy(x_hbm.at[pl.ds(n0, S_LEN - n0)], x_v.at[pl.ds(n0, S_LEN - n0)], sems.at[4 * RING + 1])
    b_cps = [pltpu.make_async_copy(src, dst, sems.at[4 * RING + 2])
             for src, dst in ((w1_hbm, w1), (w2_hbm, w2), (w3_hbm, w3), (w4_hbm, w4))]
    x_cp0.start()
    for p in range(RING):
        for cp in pair_copies(p):
            cp.start()

    xs[pl.ds(XS_DUMMY, SEG), :] = jnp.zeros((SEG, D), f32)
    lnx[pl.ds(XS_DUMMY, SEG), :] = jnp.zeros((SEG, D), f32)
    ybuf[pl.ds(XS_DUMMY, SEG), :] = jnp.zeros((SEG, D), f32)
    hbuf[pl.ds(0, HB_PAD), :] = jnp.zeros((HB_PAD, D), f32)
    hbuf[pl.ds(HB_PAD + S_LEN, HB_ROWS - HB_PAD - S_LEN), :] = jnp.zeros((HB_ROWS - HB_PAD - S_LEN, D), f32)
    m0 = mem0_ref[...].astype(f32)
    mem[pl.ds(0, M_MEM), :] = m0
    mem[pl.ds(M_MEM, M_MEM), :] = m0
    x_cp0.wait()
    xf0 = x_v[pl.ds(0, n0), :].astype(f32)
    ln0 = _ln(xf0)
    xs[pl.ds(0, n0), :] = xf0
    lnx[pl.ds(0, n0), :] = ln0

    lane128 = lax.broadcasted_iota(jnp.int32, (L, 128), 1)
    lo64 = lane128 < 64
    l80 = lax.broadcasted_iota(jnp.int32, (L, 2 * L), 1)
    row = lax.broadcasted_iota(jnp.int32, (L, 2 * L), 0)
    ha = l80 < L
    key = jnp.where(ha, l80, l80 - L)
    allowed = (row < M_MEM) | (row >= key)
    scale = np.float32(E ** -0.5)
    z40 = jnp.zeros((L, 128), f32)
    lane32 = lax.broadcasted_iota(jnp.int32, (SEG, 128), 1)

    def seg_row(seg, dummy=XS_DUMMY):
        valid = jnp.logical_and(seg >= 0, seg < NSEG)
        return pl.multiple_of(jnp.where(valid, seg * SEG, dummy), 8)

    def blk(u):
        t0 = jnp.concatenate([u[:, 0:128], z40], axis=0)
        u1 = u[:, 128:256]
        t1 = jnp.concatenate([jnp.where(lo64, u1, 0.), jnp.where(lo64, 0., u1)], axis=0)
        t2 = jnp.concatenate([z40, u[:, 256:384]], axis=0)
        return jnp.concatenate([t0, t1, t2], axis=1).astype(bf16)

    def softmax_parts(s):
        xm = jnp.where(allowed, s * scale, np.float32(-1e9))
        m0_ = jnp.max(jnp.where(ha, xm, NEG), axis=1, keepdims=True)
        m1_ = jnp.max(jnp.where(ha, NEG, xm), axis=1, keepdims=True)
        pe = jnp.exp(xm - jnp.where(ha, m0_, m1_))
        i0 = 1.0 / jnp.sum(jnp.where(ha, pe, 0.), axis=1, keepdims=True)
        i1 = 1.0 / jnp.sum(jnp.where(ha, 0., pe), axis=1, keepdims=True)
        return pe, i0, i1

    def pv(parts, vb):
        pe, i0, i1 = parts
        o = _dot(pe, vb, NN)
        return jnp.concatenate([o[:, 0:128] * i0, o[:, 128:256] * jnp.where(lo64, i0, i1), o[:, 256:384] * i1],
                               axis=1)

    def make_stages(a_slots, ba_segs, bb_slots, pre_row=None, first_b=None):
        na = len(a_slots)
        st = {}
        a_rows = [seg_row(s) for s, _ in a_slots]
        ba_rows = [seg_row(s) for s in ba_segs]
        bb_rows = [seg_row(s) for s, _ in bb_slots]
        bah_rows = [seg_row(s, HB_DUMMY) + HB_PAD for s in ba_segs]
        bbh_rows = [seg_row(s, HB_DUMMY) for s, _ in bb_slots]
        fns = {}

        def stage(f):
            fns[f.__name__] = f
            return f

        if na:
            parts = []
            for l, ((_, mr), r) in enumerate(zip(a_slots, a_rows)):
                parts.append(mem[pl.ds(mr, M_MEM), :])
                if not (l == 0 and pre_row is not None):
                    parts.append(lnx[pl.ds(r, SEG), :])
            h = jnp.concatenate(parts, axis=0).astype(bf16 if na == 2 else f32)

        def proj(m, p):
            r = _dot(h, pltpu.bitcast(wn[p, m], bf16), NN)
            if pre_row is None:
                return [r[L * l:L * l + L] for l in range(na)]
            tok = pre[m, pl.ds(pre_row, SEG), pl.ds(PW * p, PW)]
            return [jnp.concatenate([r[0:M_MEM], tok], axis=0), r[M_MEM:M_MEM + L]]

        @stage
        def a_k(p):
            st['k', p] = [blk(k) for k in proj(0, p)]

        @stage
        def a_q(p):
            st['q', p] = proj(1, p)

        @stage
        def a_v(p):
            st['v', p] = [blk(v) for v in proj(2, p)]

        @stage
        def a_s(p):
            qs, ks = st.pop(('q', p)), st.pop(('k', p))
            st['p', p] = [softmax_parts(_dot(qs[l], ks[l], NT)) for l in range(na)]

        @stage
        def a_pv(p):
            ps, vs = st.pop(('p', p)), st.pop(('v', p))
            o = jnp.concatenate([pv(ps[l], vs[l]) for l in range(na)], axis=0)
            st['o', p] = o.astype(bf16) if na == 2 else o

        @stage
        def a_out(p):
            r = _dot(st.pop(('o', p)), pltpu.bitcast(won[p], bf16), NN)
            st['acc'] = r if 'acc' not in st else st['acc'] + r

        @stage
        def a_fin():
            acc = st.pop('acc')
            for l, ((_, mr), r) in enumerate(zip(a_slots, a_rows)):
                mem[pl.ds(mr, M_MEM), :] = acc[L * l:L * l + M_MEM]
                xs[pl.ds(r, SEG), :] = xs[pl.ds(r, SEG), :] + acc[L * l + M_MEM:L * l + L]

        @stage
        def x_ln():
            seg = a_slots[0][0] + NPRE
            src = pl.multiple_of(jnp.minimum(seg, NSEG - 1) * SEG, SEG)
            xf = x_v[pl.ds(src, SEG), :].astype(f32)
            r = seg_row(seg)
            xs[pl.ds(r, SEG), :] = xf
            lnx[pl.ds(r, SEG), :] = _ln(xf)

        @stage
        def b_wait():
            @pl.when(first_b)
            def _():
                for cp in b_cps:
                    cp.wait()

        @stage
        def b_pre():
            xa = jnp.concatenate([xs[pl.ds(r, SEG), :] for r in ba_rows], axis=0)
            y = _ln(xa)
            for l, r in enumerate(ba_rows):
                ybuf[pl.ds(r, SEG), :] = y[SEG * l:SEG * l + SEG]
            st['y2'] = _ln(y).astype(bf16)

        @stage
        def b_mm1():
            hh = _gelu(_dot(st.pop('y2'), w1[...], NN))
            for l, r in enumerate(bah_rows):
                hbuf[pl.ds(r, SEG), :] = hh[SEG * l:SEG * l + SEG]

        @stage
        def b_shift():
            parts = []
            for r in bbh_rows:
                win = hbuf[pl.ds(r, SEG + 2 * HB_PAD), :]

                def sh(d, c):
                    return win[HB_PAD + d:HB_PAD + d + SEG, 128 * c:128 * c + 128]
                parts.append(jnp.concatenate([
                    sh(-1, 0),
                    jnp.where(lane32 < 32, sh(-1, 1), sh(1, 1)),
                    jnp.where(lane32 < 64, sh(1, 2), sh(-2, 2)),
                    jnp.where(lane32 < 96, sh(-2, 3), sh(2, 3)),
                    sh(2, 4)], axis=1))
            st['hsft'] = jnp.concatenate(parts, axis=0).astype(bf16)

        @stage
        def b_mm2():
            hs = _dot(st.pop('hsft'), w2[...], NN)
            y = jnp.concatenate([ybuf[pl.ds(r, SEG), :] for r in bb_rows], axis=0)
            x1 = y + hs
            xa = jnp.concatenate([xs[pl.ds(r, SEG), :] for r in bb_rows], axis=0)
            st['res'] = xa + x1
            st['z'] = _ln(x1).astype(bf16)

        @stage
        def b_mm3(c):
            st['g', c] = _gelu(_dot(st['z'], w3[:, pl.ds(512 * c, 512)], NN)).astype(bf16)

        @stage
        def b_mm4(c):
            st['res'] = st['res'] + _dot(st.pop(('g', c)), w4[pl.ds(512 * c, 512), :], NN)

        @stage
        def b_fin():
            o = st.pop('res')
            for l, ((_, final), r) in enumerate(zip(bb_slots, bb_rows)):
                ol = o[SEG * l:SEG * l + SEG]
                if not isinstance(final, bool):
                    rf = pl.multiple_of(jnp.where(final, r, XS_DUMMY), 8)
                    rn = pl.multiple_of(jnp.where(final, XS_DUMMY, r), 8)
                    outs[pl.ds(rf, SEG), :] = ol.astype(bf16)
                    xs[pl.ds(rn, SEG), :] = ol
                    lnx[pl.ds(rn, SEG), :] = _ln(ol)
                elif final:
                    outs[pl.ds(r, SEG), :] = ol.astype(bf16)
                else:
                    xs[pl.ds(r, SEG), :] = ol
                    lnx[pl.ds(r, SEG), :] = _ln(ol)

        def run(name):
            if ':' in name:
                n, a = name.split(':')
                fns[n](int(a))
            else:
                fns[name]()
        return run

    def run_order(run, order):
        offs = [o for _, o in order['iter']]
        for i in range(-max(offs), NP - min(offs)):
            sched = list(order.get((i, 'pre'), []))
            for name, o in order['iter']:
                if 0 <= i + o < NP:
                    sched.append('a_%s:%d' % (name, i + o))
                    sched += order.get((i, name), [])
            sched += order.get((i, 'end'), [])
            for s in sched:
                run(s)

    def b_slots(t):
        return ([t - 1, t - LAG - 1], [(t - 2, False), (t - LAG - 2, True)])

    h0 = jnp.concatenate([m0, ln0[0:SEG], ln0[PRE0 * SEG:n0]], axis=0)

    def attend0(p):
        c = pl.ds(pl.multiple_of(p * PW, PW), PW)
        st = {}
        k0, q0, v0 = (pre[m, pl.ds(0, L), c] for m in range(3))

        def a_s():
            st['p'] = softmax_parts(_dot(q0, blk(k0), NT))

        def a_pv():
            st['o'] = pv(st['p'], blk(v0))

        def a_out(acc):
            return acc + _dot(st['o'], pltpu.bitcast(won[p], bf16), NN)
        return a_s, a_pv, a_out

    for m in range(3):
        pre[m, pl.ds(0, L), pl.ds(0, PW)] = jnp.zeros((L, PW), f32)

    def first(p, acc):
        cps = pair_copies(p)
        slot = p % RING
        c = pl.ds(pl.multiple_of(p * PW, PW), PW)
        a_s, a_pv, a_out = attend0(jnp.maximum(p - 1, 0))

        st = {'acc': acc}

        def proj0(m):
            pre[m, :, c] = _dot(h0, stg[slot, m], NT)

        def retile(m):
            w = stg[slot, m]
            if m < 3:
                wn[p, m] = pltpu.bitcast(jnp.transpose(w), jnp.uint32)
            else:
                won[p] = pltpu.bitcast(w, jnp.uint32)

        def out0():
            st['acc'] = a_out(st['acc'])
        ops = {'k': lambda: proj0(0), 'q': lambda: proj0(1), 'v': lambda: proj0(2),
               'tk': lambda: retile(0), 'tq': lambda: retile(1), 'tv': lambda: retile(2), 'to': lambda: retile(3),
               'wk': cps[0].wait, 'wq': cps[1].wait, 'wv': cps[2].wait, 'wo': cps[3].wait,
               's': a_s, 'pv': a_pv, 'out': out0}
        for name in ORDER_V0:
            ops[name]()
        acc = st['acc']

        @pl.when(p + RING < NP)
        def _():
            for cp in pair_copies(jnp.minimum(p + RING, NP - 1)):
                cp.start()

        @pl.when(p + RING == NP)
        def _():
            for cp in b_cps:
                cp.start()
            x_cp.start()
        return acc
    acc0 = lax.fori_loop(0, NP, first, jnp.zeros((L, D), f32))
    a_s, a_pv, a_out = attend0(NP - 1)
    a_s()
    a_pv()
    acc0 = a_out(acc0)
    mem[pl.ds(0, M_MEM), :] = acc0[0:M_MEM]
    xs[pl.ds(0, SEG), :] = xs[pl.ds(0, SEG), :] + acc0[M_MEM:L]

    def step(t, carry):
        pre_on = jnp.logical_and(t >= PRE0, t < PRE0 + NPRE)
        full = jnp.logical_and(t >= PRE0 + NPRE, t < NSEG)
        single = jnp.logical_or(t < LAG, t >= NSEG)

        @pl.when(t == LAG)
        def _():
            x_cp.wait()

        @pl.when(full)
        def _():
            ba, bb = b_slots(t)
            run_order(make_stages([(t, 0), (t - LAG, M_MEM)], ba, bb), ORDER_V80)

        @pl.when(pre_on)
        def _():
            ba, bb = b_slots(t)
            pr = pl.multiple_of(L + (jnp.clip(t, PRE0, PRE0 + NPRE - 1) - PRE0) * SEG, 8)
            run_order(make_stages([(t, 0), (t - LAG, M_MEM)], ba, bb, pre_row=pr), ORDER_V48)

        @pl.when(single)
        def _():
            early = t < LAG
            seg = jnp.where(early, t, t - LAG)
            mr = pl.multiple_of(jnp.where(early, 0, M_MEM), M_MEM)
            ba = jnp.where(t <= NSEG, t - 1, t - LAG - 2)
            bb = jnp.where(t <= NSEG + 1, t - 2, NSEG - 5)
            run_order(make_stages([(seg, mr)], [ba], [(bb, t > NSEG + 1)], first_b=(t == 1)), ORDER_V40)
        return carry
    lax.fori_loop(1, NSEG + LAG, step, 0)

    n_done = NSEG - 4
    cp_a = pltpu.make_async_copy(outs.at[pl.ds(0, n_done * SEG)], out_hbm.at[pl.ds(0, n_done * SEG)], osem.at[0])
    cp_a.start()
    run = make_stages([], [NSEG - 2, NSEG - 1], [(NSEG - 4, True), (NSEG - 3, True)])
    run2 = make_stages([], [], [(NSEG - 2, True), (NSEG - 1, True)])
    for s in ['b_pre', 'b_mm1', 'b_shift', 'b_mm2']:
        run(s)
    for s in ['b_shift', 'b_mm2']:
        run2(s)
    for c in range(3):
        run('b_mm3:%d' % c)
        run2('b_mm3:%d' % c)
    for c in range(3):
        run('b_mm4:%d' % c)
        run2('b_mm4:%d' % c)
    run('b_fin')
    run2('b_fin')
    cp_b = pltpu.make_async_copy(outs.at[pl.ds(n_done * SEG, 4 * SEG)], out_hbm.at[pl.ds(n_done * SEG, 4 * SEG)],
                                 osem.at[1])
    cp_b.start()
    cp_a.wait()
    cp_b.wait()


@functools.partial(jax.jit, static_argnames=("A_seg_len",))
def pallas_interleave_layers__memory_aug_recurrent_mem_tr__mixer_s_mlp__prompt_kernel(
        A_x, A_mem0, A_Wq, A_Wk, A_Wv, A_Wo, A_seg_len, B_x, B_w1, B_w2, B_w3, B_w4):
    del B_x
    assert A_seg_len == SEG and A_x.shape == (1, S_LEN, D) and A_Wq.shape == (D, H, E)
    x = A_x.reshape(S_LEN, D)
    mem0 = A_mem0.reshape(M_MEM, D)
    wqt, wkt, wvt = (jnp.transpose(w, (1, 2, 0)).reshape(H * E, D) for w in (A_Wq, A_Wk, A_Wv))
    wo = A_Wo.reshape(H * E, D)
    any_spec = pl.BlockSpec(memory_space=pl.ANY)
    out = pl.pallas_call(
        _kernel,
        out_shape=jax.ShapeDtypeStruct((S_LEN, D), bf16),
        in_specs=[any_spec, pl.BlockSpec(memory_space=pltpu.VMEM)] + [any_spec] * 8,
        out_specs=any_spec,
        scratch_shapes=[
            pltpu.VMEM((S_LEN, D), bf16),
            pltpu.VMEM((RING, 4, PW, D), bf16),
            pltpu.VMEM((NP, 3, D // 2, PW), jnp.uint32),
            pltpu.VMEM((NP, PW // 2, D), jnp.uint32),
            pltpu.VMEM((D, D), bf16), pltpu.VMEM((D, D), bf16),
            pltpu.VMEM((D, F), bf16), pltpu.VMEM((F, D), bf16),
            pltpu.VMEM((XS_ROWS, D), f32), pltpu.VMEM((XS_ROWS, D), f32),
            pltpu.VMEM((XS_ROWS, D), f32),
            pltpu.VMEM((HB_ROWS, D), f32),
            pltpu.VMEM((2 * M_MEM, D), f32),
            pltpu.VMEM((XS_ROWS, D), bf16),
            pltpu.VMEM((3, PRE_ROWS, H * E), f32),
            pltpu.SemaphoreType.DMA((4 * RING + 3,)),
            pltpu.SemaphoreType.DMA((2,)),
        ],
        compiler_params=pltpu.CompilerParams(vmem_limit_bytes=120 * 1024 * 1024),
        name="mem_mixer",
    )(x, mem0, wqt, wkt, wvt, wo, B_w1, B_w2, B_w3, B_w4)
    return out.reshape(1, S_LEN, D)
```

```python
import functools

import jax
import jax.numpy as jnp
import numpy as np
from jax import lax
import jax.experimental.pallas as pl
import jax.experimental.pallas.tpu as pltpu

f32 = jnp.float32
bf16 = jnp.bfloat16

S_LEN, D, H, E = 2048, 640, 32, 192
M_MEM, SEG = 8, 32
L = M_MEM + SEG
NSEG = S_LEN // SEG
NP = H // 2
PW = 2 * E
F = 1536
LAG = 3
RING = 4
PRE0, NPRE = LAG, 8
PRE_ROWS = L + NPRE * SEG
EPS = 1e-5
NEG = -1e30

NT = (((1,), (1,)), ((), ()))
NN = (((1,), (0,)), ((), ()))


def _dot(a, b, dims):
    return lax.dot_general(a, b, dims, preferred_element_type=f32)


def _ln(x):
    m = jnp.mean(x, axis=-1, keepdims=True)
    xc = x - m
    v = jnp.mean(xc * xc, axis=-1, keepdims=True)
    return xc * lax.rsqrt(v + EPS)


def _gelu(x):
    c = np.float32(np.sqrt(2.0 / np.pi))
    return 0.5 * x * (1.0 + jnp.tanh(c * (x + np.float32(0.044715) * (x * x * x))))


XS_DUMMY = S_LEN
XS_ROWS = S_LEN + SEG
HB_PAD = 8
HB_DUMMY = S_LEN + 2 * HB_PAD
HB_ROWS = HB_DUMMY + SEG + 2 * HB_PAD

ORDER_V0 = ['wk', 'wq', 'wv', 'wo', 's', 'to', 'tk', 'k', 'pv', 'tq', 'q', 'out', 'tv', 'v']
ORDER_TAIL = [(0, 'b_pre'), (0, 'b_mm1'), (1, 'b_shift'), (0, 'b_shift'), (0, 'b_mm2'), (1, 'b_mm2'),
              (0, 'b_mm3:0'), (0, 'b_mm3:1'), (0, 'b_mm4:0'), (0, 'b_mm3:2'), (0, 'b_mm4:1'), (0, 'b_mm4:2'),
              (0, 'b_fin'), (1, 'b_mm3:0'), (1, 'b_mm3:1'), (1, 'b_mm3:2'), (1, 'b_mm4:0'), (1, 'b_mm4:1'),
              (1, 'b_mm4:2'), (1, 'b_fin')]
ORDER_V80 = {
    'iter': [('k', 2), ('q', 2), ('s', 1), ('v', 2), ('pv', 0), ('out', -1)],
    (-2, 'pre'): ['b_pre'], (1, 'out'): ['b_mm1'], (4, 'k'): ['b_shift'], (5, 'end'): ['b_mm2'],
    (9, 'k'): ['x_ln'], (10, 'pv'): ['b_mm3:0'], (13, 'pv'): ['b_mm3:1'], (14, 'pre'): ['b_mm4:0'],
    (14, 's'): ['b_mm3:2', 'b_mm4:1'], (14, 'pv'): ['b_mm4:2'], (15, 'out'): ['b_fin'], (16, 'out'): ['a_fin'],
}
ORDER_V48 = {
    'iter': [('k', 2), ('q', 2), ('s', 1), ('pv', 0), ('v', 2), ('out', -1)],
    (-2, 'q'): ['b_pre'], (2, 'q'): ['b_mm1'], (3, 'q'): ['b_shift'], (6, 's'): ['b_mm2'],
    (9, 'end'): ['x_ln'], (11, 'pv'): ['b_mm3:0'], (11, 'end'): ['b_mm3:1'], (14, 's'): ['b_mm4:0'],
    (15, 'out'): ['b_mm3:2', 'b_mm4:1', 'b_mm4:2'], (15, 'end'): ['b_fin'], (16, 'out'): ['a_fin'],
}
ORDER_V40 = {
    'iter': [('k', 2), ('q', 2), ('v', 2), ('s', 1), ('pv', 0), ('out', -1)],
    (-1, 'end'): ['b_pre'], (6, 'q'): ['b_wait'], (6, 'out'): ['b_mm1'], (7, 'q'): ['b_shift'],
    (9, 'pv'): ['b_mm2'], (11, 's'): ['b_mm3:0'], (12, 'q'): ['b_mm3:1'], (13, 'k'): ['b_mm3:2'],
    (13, 'pv'): ['b_mm4:0'], (14, 'pv'): ['b_mm4:1'], (15, 'pre'): ['b_mm4:2'], (16, 'pre'): ['b_fin'],
    (16, 'out'): ['a_fin'],
}


def _kernel(x_hbm, mem0_ref, wq_hbm, wk_hbm, wv_hbm, wo_hbm, w1_hbm, w2_hbm, w3_hbm, w4_hbm,
            out_hbm,
            x_v, stg, wn, won, w1, w2, w3, w4, xs, lnx, ybuf, hbuf, mem, outs, pre, sems, osem):
    def pair_copies(p):
        r = pl.ds(pl.multiple_of(p * PW, PW), PW)
        slot = p % RING
        return [pltpu.make_async_copy(src.at[r], stg.at[slot, m], sems.at[slot * 4 + m])
                for m, src in enumerate((wk_hbm, wq_hbm, wv_hbm, wo_hbm))]

    n0 = (PRE0 + NPRE) * SEG
    x_cp0 = pltpu.make_async_copy(x_hbm.at[pl.ds(0, n0)], x_v.at[pl.ds(0, n0)], sems.at[4 * RING])
    x_cp = pltpu.make_async_copy(x_hbm.at[pl.ds(n0, S_LEN - n0)], x_v.at[pl.ds(n0, S_LEN - n0)], sems.at[4 * RING + 1])
    b_cps = [pltpu.make_async_copy(src, dst, sems.at[4 * RING + 2])
             for src, dst in ((w1_hbm, w1), (w2_hbm, w2), (w3_hbm, w3), (w4_hbm, w4))]
    x_cp0.start()
    for p in range(RING):
        for cp in pair_copies(p):
            cp.start()

    xs[pl.ds(XS_DUMMY, SEG), :] = jnp.zeros((SEG, D), f32)
    lnx[pl.ds(XS_DUMMY, SEG), :] = jnp.zeros((SEG, D), f32)
    ybuf[pl.ds(XS_DUMMY, SEG), :] = jnp.zeros((SEG, D), f32)
    hbuf[pl.ds(0, HB_PAD), :] = jnp.zeros((HB_PAD, D), f32)
    hbuf[pl.ds(HB_PAD + S_LEN, HB_ROWS - HB_PAD - S_LEN), :] = jnp.zeros((HB_ROWS - HB_PAD - S_LEN, D), f32)
    m0 = mem0_ref[...].astype(f32)
    mem[pl.ds(0, M_MEM), :] = m0
    mem[pl.ds(M_MEM, M_MEM), :] = m0
    x_cp0.wait()
    xf0 = x_v[pl.ds(0, n0), :].astype(f32)
    ln0 = _ln(xf0)
    xs[pl.ds(0, n0), :] = xf0
    lnx[pl.ds(0, n0), :] = ln0

    lane128 = lax.broadcasted_iota(jnp.int32, (L, 128), 1)
    lo64 = lane128 < 64
    l80 = lax.broadcasted_iota(jnp.int32, (L, 2 * L), 1)
    row = lax.broadcasted_iota(jnp.int32, (L, 2 * L), 0)
    ha = l80 < L
    key = jnp.where(ha, l80, l80 - L)
    allowed = (row < M_MEM) | (row >= key)
    scale = np.float32(E ** -0.5)
    z40 = jnp.zeros((L, 128), f32)
    lane32 = lax.broadcasted_iota(jnp.int32, (SEG, 128), 1)

    def seg_row(seg, dummy=XS_DUMMY):
        valid = jnp.logical_and(seg >= 0, seg < NSEG)
        return pl.multiple_of(jnp.where(valid, seg * SEG, dummy), 8)

    def blk(u):
        t0 = jnp.concatenate([u[:, 0:128], z40], axis=0)
        u1 = u[:, 128:256]
        t1 = jnp.concatenate([jnp.where(lo64, u1, 0.), jnp.where(lo64, 0., u1)], axis=0)
        t2 = jnp.concatenate([z40, u[:, 256:384]], axis=0)
        return jnp.concatenate([t0, t1, t2], axis=1).astype(bf16)

    def softmax_parts(s):
        xm = jnp.where(allowed, s * scale, np.float32(-1e9))
        m0_ = jnp.max(jnp.where(ha, xm, NEG), axis=1, keepdims=True)
        m1_ = jnp.max(jnp.where(ha, NEG, xm), axis=1, keepdims=True)
        pe = jnp.exp(xm - jnp.where(ha, m0_, m1_))
        i0 = 1.0 / jnp.sum(jnp.where(ha, pe, 0.), axis=1, keepdims=True)
        i1 = 1.0 / jnp.sum(jnp.where(ha, 0., pe), axis=1, keepdims=True)
        return pe, i0, i1

    def pv(parts, vb):
        pe, i0, i1 = parts
        o = _dot(pe, vb, NN)
        return jnp.concatenate([o[:, 0:128] * i0, o[:, 128:256] * jnp.where(lo64, i0, i1), o[:, 256:384] * i1],
                               axis=1)

    def make_stages(a_slots, ba_segs, bb_slots, pre_row=None, first_b=None):
        na = len(a_slots)
        st = {}
        a_rows = [seg_row(s) for s, _ in a_slots]
        ba_rows = [seg_row(s) for s in ba_segs]
        bb_rows = [seg_row(s) for s, _ in bb_slots]
        bah_rows = [seg_row(s, HB_DUMMY) + HB_PAD for s in ba_segs]
        bbh_rows = [seg_row(s, HB_DUMMY) for s, _ in bb_slots]
        fns = {}

        def stage(f):
            fns[f.__name__] = f
            return f

        if na:
            parts = []
            for l, ((_, mr), r) in enumerate(zip(a_slots, a_rows)):
                parts.append(mem[pl.ds(mr, M_MEM), :])
                if not (l == 0 and pre_row is not None):
                    parts.append(lnx[pl.ds(r, SEG), :])
            h = jnp.concatenate(parts, axis=0).astype(bf16 if na == 2 else f32)

        def proj(m, p):
            r = _dot(h, pltpu.bitcast(wn[p, m], bf16), NN)
            if pre_row is None:
                return [r[L * l:L * l + L] for l in range(na)]
            tok = pre[m, pl.ds(pre_row, SEG), pl.ds(PW * p, PW)]
            return [jnp.concatenate([r[0:M_MEM], tok], axis=0), r[M_MEM:M_MEM + L]]

        @stage
        def a_k(p):
            st['k', p] = [blk(k) for k in proj(0, p)]

        @stage
        def a_q(p):
            st['q', p] = proj(1, p)

        @stage
        def a_v(p):
            st['v', p] = [blk(v) for v in proj(2, p)]

        @stage
        def a_s(p):
            qs, ks = st.pop(('q', p)), st.pop(('k', p))
            st['p', p] = [softmax_parts(_dot(qs[l], ks[l], NT)) for l in range(na)]

        @stage
        def a_pv(p):
            ps, vs = st.pop(('p', p)), st.pop(('v', p))
            o = jnp.concatenate([pv(ps[l], vs[l]) for l in range(na)], axis=0)
            st['o', p] = o.astype(bf16) if na == 2 else o

        @stage
        def a_out(p):
            r = _dot(st.pop(('o', p)), pltpu.bitcast(won[p], bf16), NN)
            st['acc'] = r if 'acc' not in st else st['acc'] + r

        @stage
        def a_fin():
            acc = st.pop('acc')
            for l, ((_, mr), r) in enumerate(zip(a_slots, a_rows)):
                mem[pl.ds(mr, M_MEM), :] = acc[L * l:L * l + M_MEM]
                xs[pl.ds(r, SEG), :] = xs[pl.ds(r, SEG), :] + acc[L * l + M_MEM:L * l + L]

        @stage
        def x_ln():
            seg = a_slots[0][0] + NPRE
            src = pl.multiple_of(jnp.minimum(seg, NSEG - 1) * SEG, SEG)
            xf = x_v[pl.ds(src, SEG), :].astype(f32)
            r = seg_row(seg)
            xs[pl.ds(r, SEG), :] = xf
            lnx[pl.ds(r, SEG), :] = _ln(xf)

        @stage
        def b_wait():
            @pl.when(first_b)
            def _():
                for cp in b_cps:
                    cp.wait()

        @stage
        def b_pre():
            xa = jnp.concatenate([xs[pl.ds(r, SEG), :] for r in ba_rows], axis=0)
            y = _ln(xa)
            for l, r in enumerate(ba_rows):
                ybuf[pl.ds(r, SEG), :] = y[SEG * l:SEG * l + SEG]
            st['y2'] = _ln(y).astype(bf16)

        @stage
        def b_mm1():
            hh = _gelu(_dot(st.pop('y2'), w1[...], NN))
            for l, r in enumerate(bah_rows):
                hbuf[pl.ds(r, SEG), :] = hh[SEG * l:SEG * l + SEG]

        @stage
        def b_shift():
            parts = []
            for r in bbh_rows:
                win = hbuf[pl.ds(r, SEG + 2 * HB_PAD), :]

                def sh(d, c):
                    return win[HB_PAD + d:HB_PAD + d + SEG, 128 * c:128 * c + 128]
                parts.append(jnp.concatenate([
                    sh(-1, 0),
                    jnp.where(lane32 < 32, sh(-1, 1), sh(1, 1)),
                    jnp.where(lane32 < 64, sh(1, 2), sh(-2, 2)),
                    jnp.where(lane32 < 96, sh(-2, 3), sh(2, 3)),
                    sh(2, 4)], axis=1))
            st['hsft'] = jnp.concatenate(parts, axis=0).astype(bf16)

        @stage
        def b_mm2():
            hs = _dot(st.pop('hsft'), w2[...], NN)
            y = jnp.concatenate([ybuf[pl.ds(r, SEG), :] for r in bb_rows], axis=0)
            x1 = y + hs
            xa = jnp.concatenate([xs[pl.ds(r, SEG), :] for r in bb_rows], axis=0)
            st['res'] = xa + x1
            st['z'] = _ln(x1).astype(bf16)

        @stage
        def b_mm3(c):
            st['g', c] = _gelu(_dot(st['z'], w3[:, pl.ds(512 * c, 512)], NN)).astype(bf16)

        @stage
        def b_mm4(c):
            st['res'] = st['res'] + _dot(st.pop(('g', c)), w4[pl.ds(512 * c, 512), :], NN)

        @stage
        def b_fin():
            o = st.pop('res')
            for l, ((_, final), r) in enumerate(zip(bb_slots, bb_rows)):
                ol = o[SEG * l:SEG * l + SEG]
                if final is True:
                    outs[pl.ds(r, SEG), :] = ol.astype(bf16)
                elif final is False:
                    xs[pl.ds(r, SEG), :] = ol
                    lnx[pl.ds(r, SEG), :] = _ln(ol)
                else:
                    rf = pl.multiple_of(jnp.where(final, r, XS_DUMMY), 8)
                    rn = pl.multiple_of(jnp.where(final, XS_DUMMY, r), 8)
                    outs[pl.ds(rf, SEG), :] = ol.astype(bf16)
                    xs[pl.ds(rn, SEG), :] = ol
                    lnx[pl.ds(rn, SEG), :] = _ln(ol)

        def run(name):
            if ':' in name:
                n, a = name.split(':')
                fns[n](int(a))
            else:
                fns[name]()
        return run

    def run_order(run, order):
        offs = [o for _, o in order['iter']]
        for i in range(-max(offs), NP - min(offs)):
            sched = list(order.get((i, 'pre'), []))
            for name, o in order['iter']:
                if 0 <= i + o < NP:
                    sched.append('a_%s:%d' % (name, i + o))
                    sched += order.get((i, name), [])
            sched += order.get((i, 'end'), [])
            for s in sched:
                run(s)

    def b_slots(t):
        return ([t - 1, t - LAG - 1], [(t - 2, False), (t - LAG - 2, True)])

    h0 = jnp.concatenate([m0, ln0[0:SEG], ln0[PRE0 * SEG:n0]], axis=0)

    def attend0(p):
        c = pl.ds(pl.multiple_of(p * PW, PW), PW)
        st = {}
        k0, q0, v0 = (pre[m, pl.ds(0, L), c] for m in range(3))

        def a_s():
            st['p'] = softmax_parts(_dot(q0, blk(k0), NT))

        def a_pv():
            st['o'] = pv(st['p'], blk(v0))

        def a_out(acc):
            return acc + _dot(st['o'], pltpu.bitcast(won[p], bf16), NN)
        return a_s, a_pv, a_out

    for m in range(3):
        pre[m, pl.ds(0, L), pl.ds(0, PW)] = jnp.zeros((L, PW), f32)

    def first(p, acc):
        cps = pair_copies(p)
        slot = p % RING
        c = pl.ds(pl.multiple_of(p * PW, PW), PW)
        a_s, a_pv, a_out = attend0(jnp.maximum(p - 1, 0))
        st = {'acc': acc}

        def proj0(m):
            pre[m, :, c] = _dot(h0, stg[slot, m], NT)

        def retile(m):
            w = stg[slot, m]
            if m < 3:
                wn[p, m] = pltpu.bitcast(jnp.transpose(w), jnp.uint32)
            else:
                won[p] = pltpu.bitcast(w, jnp.uint32)

        def out0():
            st['acc'] = a_out(st['acc'])
        ops = {'k': lambda: proj0(0), 'q': lambda: proj0(1), 'v': lambda: proj0(2),
               'tk': lambda: retile(0), 'tq': lambda: retile(1), 'tv': lambda: retile(2), 'to': lambda: retile(3),
               'wk': cps[0].wait, 'wq': cps[1].wait, 'wv': cps[2].wait, 'wo': cps[3].wait,
               's': a_s, 'pv': a_pv, 'out': out0}
        for name in ORDER_V0:
            ops[name]()

        @pl.when(p + RING < NP)
        def _():
            for cp in pair_copies(jnp.minimum(p + RING, NP - 1)):
                cp.start()

        @pl.when(p + RING == NP)
        def _():
            for cp in b_cps:
                cp.start()
            x_cp.start()
        return st['acc']
    acc0 = lax.fori_loop(0, NP, first, jnp.zeros((L, D), f32))
    a_s, a_pv, a_out = attend0(NP - 1)
    a_s()
    a_pv()
    acc0 = a_out(acc0)
    mem[pl.ds(0, M_MEM), :] = acc0[0:M_MEM]
    xs[pl.ds(0, SEG), :] = xs[pl.ds(0, SEG), :] + acc0[M_MEM:L]

    def step(t, carry):
        pre_on = jnp.logical_and(t >= PRE0, t < PRE0 + NPRE)
        full = jnp.logical_and(t >= PRE0 + NPRE, t < NSEG)
        single = jnp.logical_or(t < LAG, t >= NSEG)

        @pl.when(t == LAG)
        def _():
            x_cp.wait()

        @pl.when(full)
        def _():
            ba, bb = b_slots(t)
            run_order(make_stages([(t, 0), (t - LAG, M_MEM)], ba, bb), ORDER_V80)

        @pl.when(pre_on)
        def _():
            ba, bb = b_slots(t)
            pr = pl.multiple_of(L + (jnp.clip(t, PRE0, PRE0 + NPRE - 1) - PRE0) * SEG, 8)
            run_order(make_stages([(t, 0), (t - LAG, M_MEM)], ba, bb, pre_row=pr), ORDER_V48)

        @pl.when(single)
        def _():
            early = t < LAG
            seg = jnp.where(early, t, t - LAG)
            mr = pl.multiple_of(jnp.where(early, 0, M_MEM), M_MEM)
            ba = jnp.where(t <= NSEG, t - 1, t - LAG - 2)
            bb = jnp.where(t <= NSEG + 1, t - 2, NSEG - 5)
            run_order(make_stages([(seg, mr)], [ba], [(bb, t > NSEG + 1)], first_b=(t == 1)), ORDER_V40)
        return carry
    lax.fori_loop(1, NSEG + LAG, step, 0)

    n_done = NSEG - 4
    cp_a = pltpu.make_async_copy(outs.at[pl.ds(0, n_done * SEG)], out_hbm.at[pl.ds(0, n_done * SEG)], osem.at[0])
    cp_a.start()
    runs = (make_stages([], [NSEG - 2, NSEG - 1], [(NSEG - 4, True), (NSEG - 3, True)]),
            make_stages([], [], [(NSEG - 2, True), (NSEG - 1, True)]))
    for which, name in ORDER_TAIL:
        runs[which](name)
    cp_b = pltpu.make_async_copy(outs.at[pl.ds(n_done * SEG, 4 * SEG)], out_hbm.at[pl.ds(n_done * SEG, 4 * SEG)],
                                 osem.at[1])
    cp_b.start()
    cp_a.wait()
    cp_b.wait()


@functools.partial(jax.jit, static_argnames=("A_seg_len",))
def pallas_interleave_layers__memory_aug_recurrent_mem_tr__mixer_s_mlp__prompt_kernel(
        A_x, A_mem0, A_Wq, A_Wk, A_Wv, A_Wo, A_seg_len, B_x, B_w1, B_w2, B_w3, B_w4):
    del B_x
    assert A_seg_len == SEG and A_x.shape == (1, S_LEN, D) and A_Wq.shape == (D, H, E)
    x = A_x.reshape(S_LEN, D)
    mem0 = A_mem0.reshape(M_MEM, D)
    wqt, wkt, wvt = (jnp.transpose(w, (1, 2, 0)).reshape(H * E, D) for w in (A_Wq, A_Wk, A_Wv))
    wo = A_Wo.reshape(H * E, D)
    any_spec = pl.BlockSpec(memory_space=pl.ANY)
    out = pl.pallas_call(
        _kernel,
        out_shape=jax.ShapeDtypeStruct((S_LEN, D), bf16),
        in_specs=[any_spec, pl.BlockSpec(memory_space=pltpu.VMEM)] + [any_spec] * 8,
        out_specs=any_spec,
        scratch_shapes=[
            pltpu.VMEM((S_LEN, D), bf16),
            pltpu.VMEM((RING, 4, PW, D), bf16),
            pltpu.VMEM((NP, 3, D // 2, PW), jnp.uint32),
            pltpu.VMEM((NP, PW // 2, D), jnp.uint32),
            pltpu.VMEM((D, D), bf16), pltpu.VMEM((D, D), bf16),
            pltpu.VMEM((D, F), bf16), pltpu.VMEM((F, D), bf16),
            pltpu.VMEM((XS_ROWS, D), f32), pltpu.VMEM((XS_ROWS, D), f32),
            pltpu.VMEM((XS_ROWS, D), f32),
            pltpu.VMEM((HB_ROWS, D), f32),
            pltpu.VMEM((2 * M_MEM, D), f32),
            pltpu.VMEM((XS_ROWS, D), bf16),
            pltpu.VMEM((3, PRE_ROWS, H * E), f32),
            pltpu.SemaphoreType.DMA((4 * RING + 3,)),
            pltpu.SemaphoreType.DMA((2,)),
        ],
        compiler_params=pltpu.CompilerParams(vmem_limit_bytes=120 * 1024 * 1024),
        name="mem_mixer",
    )(x, mem0, wqt, wkt, wvt, wo, B_w1, B_w2, B_w3, B_w4)
    return out.reshape(1, S_LEN, D)
```

```python
import functools

import jax
import jax.numpy as jnp
import numpy as np
from jax import lax
import jax.experimental.pallas as pl
import jax.experimental.pallas.tpu as pltpu

f32 = jnp.float32
bf16 = jnp.bfloat16

S_LEN, D, H, E = 2048, 640, 32, 192
M_MEM, SEG = 8, 32
L = M_MEM + SEG
NSEG = S_LEN // SEG
NP = H // 2
PW = 2 * E
F = 1536
LAG = 3
RING = 4
PRE0, NPRE = LAG, 8
PRE_ROWS = L + NPRE * SEG
EPS = 1e-5
NEG = -1e30

NT = (((1,), (1,)), ((), ()))
NN = (((1,), (0,)), ((), ()))


def _dot(a, b, dims):
    return lax.dot_general(a, b, dims, preferred_element_type=f32)


def _ln(x):
    m = jnp.mean(x, axis=-1, keepdims=True)
    xc = x - m
    v = jnp.mean(xc * xc, axis=-1, keepdims=True)
    return xc * lax.rsqrt(v + EPS)


def _gelu(x):
    c = np.float32(np.sqrt(2.0 / np.pi))
    return 0.5 * x * (1.0 + jnp.tanh(c * (x + np.float32(0.044715) * (x * x * x))))


XS_DUMMY = S_LEN
XS_ROWS = S_LEN + SEG
HB_PAD = 8
HB_DUMMY = S_LEN + 2 * HB_PAD
HB_ROWS = HB_DUMMY + SEG + 2 * HB_PAD

ORDER_V0 = ['wk', 'wq', 'wv', 'wo', 's', 'to', 'tk', 'k', 'pv', 'tq', 'q', 'out', 'tv', 'v']
ORDER_TAIL = [(0, 'b_pre'), (0, 'b_mm1'), (1, 'b_shift'), (0, 'b_shift'), (0, 'b_mm2'), (1, 'b_mm2'),
              (0, 'b_mm3:0'), (0, 'b_mm3:1'), (0, 'b_mm4:0'), (0, 'b_mm3:2'), (0, 'b_mm4:1'), (0, 'b_mm4:2'),
              (0, 'b_fin'), (1, 'b_mm3:0'), (1, 'b_mm3:1'), (1, 'b_mm3:2'), (1, 'b_mm4:0'), (1, 'b_mm4:1'),
              (1, 'b_mm4:2'), (1, 'b_fin')]
ORDER_V80 = {
    'iter': [('k', 2), ('q', 2), ('s', 1), ('v', 2), ('pv', 0), ('out', -1)],
    (-2, 'pre'): ['b_pre'], (1, 'out'): ['b_mm1'], (4, 'k'): ['b_shift'], (5, 'end'): ['b_mm2'],
    (9, 'k'): ['x_ln'], (10, 'pv'): ['b_mm3:0'], (13, 'pv'): ['b_mm3:1'], (14, 'pre'): ['b_mm4:0'],
    (14, 's'): ['b_mm3:2', 'b_mm4:1'], (14, 'pv'): ['b_mm4:2'], (15, 'out'): ['b_fin'], (16, 'out'): ['a_fin'],
}
ORDER_V48 = {
    'iter': [('k', 2), ('q', 2), ('s', 1), ('pv', 0), ('v', 2), ('out', -1)],
    (-2, 'q'): ['b_pre'], (2, 'q'): ['b_mm1'], (3, 'q'): ['b_shift'], (6, 's'): ['b_mm2'],
    (9, 'end'): ['x_ln'], (11, 'pv'): ['b_mm3:0'], (11, 'end'): ['b_mm3:1'], (14, 's'): ['b_mm4:0'],
    (15, 'out'): ['b_mm3:2', 'b_mm4:1', 'b_mm4:2'], (15, 'end'): ['b_fin'], (16, 'out'): ['a_fin'],
}
ORDER_V40 = {
    'iter': [('k', 2), ('q', 2), ('v', 2), ('s', 1), ('pv', 0), ('out', -1)],
    (-1, 'end'): ['b_pre'], (6, 'q'): ['b_wait'], (6, 'out'): ['b_mm1'], (7, 'q'): ['b_shift'],
    (9, 'pv'): ['b_mm2'], (11, 's'): ['b_mm3:0'], (12, 'q'): ['b_mm3:1'], (13, 'k'): ['b_mm3:2'],
    (13, 'pv'): ['b_mm4:0'], (14, 'pv'): ['b_mm4:1'], (15, 'pre'): ['b_mm4:2'], (16, 'pre'): ['b_fin'],
    (16, 'out'): ['a_fin'],
}


def _kernel(x_hbm, mem0_ref, wq_hbm, wk_hbm, wv_hbm, wo_hbm, w1_hbm, w2_hbm, w3_hbm, w4_hbm,
            out_hbm,
            x_v, stg, wn, won, w1, w2, w3, w4, xs, lnx, ybuf, hbuf, mem, outs, pre, sems, osem):
    def pair_copies(p):
        r = pl.ds(pl.multiple_of(p * PW, PW), PW)
        slot = p % RING
        return [pltpu.make_async_copy(src.at[r], stg.at[slot, m], sems.at[slot * 4 + m])
                for m, src in enumerate((wk_hbm, wq_hbm, wv_hbm, wo_hbm))]

    n0 = (PRE0 + NPRE) * SEG
    x_cp0 = pltpu.make_async_copy(x_hbm.at[pl.ds(0, n0)], x_v.at[pl.ds(0, n0)], sems.at[4 * RING])
    x_cp = pltpu.make_async_copy(x_hbm.at[pl.ds(n0, S_LEN - n0)], x_v.at[pl.ds(n0, S_LEN - n0)], sems.at[4 * RING + 1])
    b_cps = [pltpu.make_async_copy(src, dst, sems.at[4 * RING + 2])
             for src, dst in ((w1_hbm, w1), (w2_hbm, w2), (w3_hbm, w3), (w4_hbm, w4))]
    x_cp0.start()
    for p in range(RING):
        for cp in pair_copies(p):
            cp.start()

    xs[pl.ds(XS_DUMMY, SEG), :] = jnp.zeros((SEG, D), f32)
    lnx[pl.ds(XS_DUMMY, SEG), :] = jnp.zeros((SEG, D), f32)
    ybuf[pl.ds(XS_DUMMY, SEG), :] = jnp.zeros((SEG, D), f32)
    hbuf[pl.ds(0, HB_PAD), :] = jnp.zeros((HB_PAD, D), f32)
    hbuf[pl.ds(HB_PAD + S_LEN, HB_ROWS - HB_PAD - S_LEN), :] = jnp.zeros((HB_ROWS - HB_PAD - S_LEN, D), f32)
    m0 = mem0_ref[...].astype(f32)
    mem[pl.ds(0, M_MEM), :] = m0
    mem[pl.ds(M_MEM, M_MEM), :] = m0
    x_cp0.wait()
    xf0 = x_v[pl.ds(0, n0), :].astype(f32)
    ln0 = _ln(xf0)
    xs[pl.ds(0, n0), :] = xf0
    lnx[pl.ds(0, n0), :] = ln0

    lane128 = lax.broadcasted_iota(jnp.int32, (L, 128), 1)
    lo64 = lane128 < 64
    l80 = lax.broadcasted_iota(jnp.int32, (L, 2 * L), 1)
    row = lax.broadcasted_iota(jnp.int32, (L, 2 * L), 0)
    ha = l80 < L
    key = jnp.where(ha, l80, l80 - L)
    allowed = (row < M_MEM) | (row >= key)
    scale = np.float32(E ** -0.5)
    z40 = jnp.zeros((L, 128), f32)
    lane32 = lax.broadcasted_iota(jnp.int32, (SEG, 128), 1)

    def seg_row(seg, dummy=XS_DUMMY):
        valid = jnp.logical_and(seg >= 0, seg < NSEG)
        return pl.multiple_of(jnp.where(valid, seg * SEG, dummy), 8)

    def blk(u):
        t0 = jnp.concatenate([u[:, 0:128], z40], axis=0)
        u1 = u[:, 128:256]
        t1 = jnp.concatenate([jnp.where(lo64, u1, 0.), jnp.where(lo64, 0., u1)], axis=0)
        t2 = jnp.concatenate([z40, u[:, 256:384]], axis=0)
        return jnp.concatenate([t0, t1, t2], axis=1).astype(bf16)

    def softmax_parts(s):
        xm = jnp.where(allowed, s * scale, np.float32(-1e9))
        m0_ = jnp.max(jnp.where(ha, xm, NEG), axis=1, keepdims=True)
        m1_ = jnp.max(jnp.where(ha, NEG, xm), axis=1, keepdims=True)
        pe = jnp.exp(xm - jnp.where(ha, m0_, m1_))
        i0 = 1.0 / jnp.sum(jnp.where(ha, pe, 0.), axis=1, keepdims=True)
        i1 = 1.0 / jnp.sum(jnp.where(ha, 0., pe), axis=1, keepdims=True)
        return pe, i0, i1

    def pv(parts, vb):
        pe, i0, i1 = parts
        o = _dot(pe, vb, NN)
        return jnp.concatenate([o[:, 0:128] * i0, o[:, 128:256] * jnp.where(lo64, i0, i1), o[:, 256:384] * i1],
                               axis=1)

    def make_stages(a_slots, ba_segs, bb_slots, pre_row=None, first_b=None):
        na = len(a_slots)
        st = {}
        a_rows = [seg_row(s) for s, _ in a_slots]
        ba_rows = [seg_row(s) for s in ba_segs]
        bb_rows = [seg_row(s) for s, _ in bb_slots]
        bah_rows = [seg_row(s, HB_DUMMY) + HB_PAD for s in ba_segs]
        bbh_rows = [seg_row(s, HB_DUMMY) for s, _ in bb_slots]
        fns = {}

        def stage(f):
            fns[f.__name__] = f
            return f

        if na:
            parts = []
            for l, ((_, mr), r) in enumerate(zip(a_slots, a_rows)):
                parts.append(mem[pl.ds(mr, M_MEM), :])
                if not (l == 0 and pre_row is not None):
                    parts.append(lnx[pl.ds(r, SEG), :])
            h = jnp.concatenate(parts, axis=0).astype(bf16 if na == 2 else f32)

        def proj(m, p):
            r = _dot(h, pltpu.bitcast(wn[p, m], bf16), NN)
            if pre_row is None:
                return [r[L * l:L * l + L] for l in range(na)]
            tok = pre[m, pl.ds(pre_row, SEG), pl.ds(PW * p, PW)]
            return [jnp.concatenate([r[0:M_MEM], tok], axis=0), r[M_MEM:M_MEM + L]]

        @stage
        def a_k(p):
            st['k', p] = [blk(k) for k in proj(0, p)]

        @stage
        def a_q(p):
            st['q', p] = proj(1, p)

        @stage
        def a_v(p):
            st['v', p] = [blk(v) for v in proj(2, p)]

        @stage
        def a_s(p):
            qs, ks = st.pop(('q', p)), st.pop(('k', p))
            st['p', p] = [softmax_parts(_dot(qs[l], ks[l], NT)) for l in range(na)]

        @stage
        def a_pv(p):
            ps, vs = st.pop(('p', p)), st.pop(('v', p))
            o = jnp.concatenate([pv(ps[l], vs[l]) for l in range(na)], axis=0)
            st['o', p] = o.astype(bf16) if na == 2 else o

        @stage
        def a_out(p):
            r = _dot(st.pop(('o', p)), pltpu.bitcast(won[p], bf16), NN)
            st['acc'] = r if 'acc' not in st else st['acc'] + r

        @stage
        def a_fin():
            acc = st.pop('acc')
            for l, ((_, mr), r) in enumerate(zip(a_slots, a_rows)):
                mem[pl.ds(mr, M_MEM), :] = acc[L * l:L * l + M_MEM]
                xs[pl.ds(r, SEG), :] = xs[pl.ds(r, SEG), :] + acc[L * l + M_MEM:L * l + L]

        @stage
        def x_ln():
            seg = a_slots[0][0] + NPRE
            src = pl.multiple_of(jnp.minimum(seg, NSEG - 1) * SEG, SEG)
            xf = x_v[pl.ds(src, SEG), :].astype(f32)
            r = seg_row(seg)
            xs[pl.ds(r, SEG), :] = xf
            lnx[pl.ds(r, SEG), :] = _ln(xf)

        @stage
        def b_wait():
            @pl.when(first_b)
            def _():
                for cp in b_cps:
                    cp.wait()

        @stage
        def b_pre():
            xa = jnp.concatenate([xs[pl.ds(r, SEG), :] for r in ba_rows], axis=0)
            y = _ln(xa)
            for l, r in enumerate(ba_rows):
                ybuf[pl.ds(r, SEG), :] = y[SEG * l:SEG * l + SEG]
            st['y2'] = _ln(y).astype(bf16)

        @stage
        def b_mm1():
            hh = _gelu(_dot(st.pop('y2'), w1[...], NN))
            for l, r in enumerate(bah_rows):
                hbuf[pl.ds(r, SEG), :] = hh[SEG * l:SEG * l + SEG]

        @stage
        def b_shift():
            parts = []
            for r in bbh_rows:
                win = hbuf[pl.ds(r, SEG + 2 * HB_PAD), :]

                def sh(d, c):
                    return win[HB_PAD + d:HB_PAD + d + SEG, 128 * c:128 * c + 128]
                parts.append(jnp.concatenate([
                    sh(-1, 0),
                    jnp.where(lane32 < 32, sh(-1, 1), sh(1, 1)),
                    jnp.where(lane32 < 64, sh(1, 2), sh(-2, 2)),
                    jnp.where(lane32 < 96, sh(-2, 3), sh(2, 3)),
                    sh(2, 4)], axis=1))
            st['hsft'] = jnp.concatenate(parts, axis=0).astype(bf16)

        @stage
        def b_mm2():
            hs = _dot(st.pop('hsft'), w2[...], NN)
            y = jnp.concatenate([ybuf[pl.ds(r, SEG), :] for r in bb_rows], axis=0)
            x1 = y + hs
            xa = jnp.concatenate([xs[pl.ds(r, SEG), :] for r in bb_rows], axis=0)
            st['res'] = xa + x1
            st['z'] = _ln(x1).astype(bf16)

        @stage
        def b_mm3(c):
            st['g', c] = _gelu(_dot(st['z'], w3[:, pl.ds(512 * c, 512)], NN)).astype(bf16)

        @stage
        def b_mm4(c):
            st['res'] = st['res'] + _dot(st.pop(('g', c)), w4[pl.ds(512 * c, 512), :], NN)

        @stage
        def b_fin():
            o = st.pop('res')
            for l, ((_, final), r) in enumerate(zip(bb_slots, bb_rows)):
                ol = o[SEG * l:SEG * l + SEG]
                if final is True:
                    outs[pl.ds(r, SEG), :] = ol.astype(bf16)
                elif final is False:
                    xs[pl.ds(r, SEG), :] = ol
                    lnx[pl.ds(r, SEG), :] = _ln(ol)
                else:
                    rf = pl.multiple_of(jnp.where(final, r, XS_DUMMY), 8)
                    rn = pl.multiple_of(jnp.where(final, XS_DUMMY, r), 8)
                    outs[pl.ds(rf, SEG), :] = ol.astype(bf16)
                    xs[pl.ds(rn, SEG), :] = ol
                    lnx[pl.ds(rn, SEG), :] = _ln(ol)

        def run(name):
            if ':' in name:
                n, a = name.split(':')
                fns[n](int(a))
            else:
                fns[name]()
        return run

    def run_order(run, order):
        offs = [o for _, o in order['iter']]
        for i in range(-max(offs), NP - min(offs)):
            sched = list(order.get((i, 'pre'), []))
            for name, o in order['iter']:
                if 0 <= i + o < NP:
                    sched.append('a_%s:%d' % (name, i + o))
                    sched += order.get((i, name), [])
            sched += order.get((i, 'end'), [])
            for s in sched:
                run(s)

    def b_slots(t):
        return ([t - 1, t - LAG - 1], [(t - 2, False), (t - LAG - 2, True)])

    h0 = jnp.concatenate([m0, ln0[0:SEG], ln0[PRE0 * SEG:n0]], axis=0)

    def attend0(p):
        c = pl.ds(pl.multiple_of(p * PW, PW), PW)
        st = {}
        k0, q0, v0 = (pre[m, pl.ds(0, L), c] for m in range(3))

        def a_s():
            st['p'] = softmax_parts(_dot(q0, blk(k0), NT))

        def a_pv():
            st['o'] = pv(st['p'], blk(v0))

        def a_out(acc):
            return acc + _dot(st['o'], pltpu.bitcast(won[p], bf16), NN)
        return a_s, a_pv, a_out

    for m in range(3):
        pre[m, pl.ds(0, L), pl.ds(0, PW)] = jnp.zeros((L, PW), f32)

    def first(p, acc):
        cps = pair_copies(p)
        slot = p % RING
        c = pl.ds(pl.multiple_of(p * PW, PW), PW)
        a_s, a_pv, a_out = attend0(jnp.maximum(p - 1, 0))
        st = {'acc': acc}

        def proj0(m):
            pre[m, :, c] = _dot(h0, stg[slot, m], NT)

        def retile(m):
            w = stg[slot, m]
            if m < 3:
                wn[p, m] = pltpu.bitcast(jnp.transpose(w), jnp.uint32)
            else:
                won[p] = pltpu.bitcast(w, jnp.uint32)

        def out0():
            st['acc'] = a_out(st['acc'])
        ops = {'k': lambda: proj0(0), 'q': lambda: proj0(1), 'v': lambda: proj0(2),
               'tk': lambda: retile(0), 'tq': lambda: retile(1), 'tv': lambda: retile(2), 'to': lambda: retile(3),
               'wk': cps[0].wait, 'wq': cps[1].wait, 'wv': cps[2].wait, 'wo': cps[3].wait,
               's': a_s, 'pv': a_pv, 'out': out0}
        for name in ORDER_V0:
            ops[name]()

        @pl.when(p + RING < NP)
        def _():
            for cp in pair_copies(jnp.minimum(p + RING, NP - 1)):
                cp.start()

        @pl.when(p + RING == NP)
        def _():
            for cp in b_cps:
                cp.start()
            x_cp.start()
        return st['acc']
    acc0 = lax.fori_loop(0, NP, first, jnp.zeros((L, D), f32))
    a_s, a_pv, a_out = attend0(NP - 1)
    a_s()
    a_pv()
    acc0 = a_out(acc0)
    mem[pl.ds(0, M_MEM), :] = acc0[0:M_MEM]
    xs[pl.ds(0, SEG), :] = xs[pl.ds(0, SEG), :] + acc0[M_MEM:L]

    def step_both(t, carry):
        ba, bb = b_slots(t)
        run_order(make_stages([(t, 0), (t - LAG, M_MEM)], ba, bb), ORDER_V80)
        return carry

    def step_both_pre(t, carry):
        ba, bb = b_slots(t)
        pr = pl.multiple_of(L + (t - PRE0) * SEG, 8)
        run_order(make_stages([(t, 0), (t - LAG, M_MEM)], ba, bb, pre_row=pr), ORDER_V48)
        return carry

    def step_single(t, carry):
        early = t < LAG
        seg = jnp.where(early, t, t - LAG)
        mr = pl.multiple_of(jnp.where(early, 0, M_MEM), M_MEM)
        ba = jnp.where(t <= NSEG, t - 1, t - LAG - 2)
        bb = jnp.where(t <= NSEG + 1, t - 2, NSEG - 5)
        run_order(make_stages([(seg, mr)], [ba], [(bb, t > NSEG + 1)], first_b=(t == 1)), ORDER_V40)
        return carry

    def phase(ph, carry):
        lax.fori_loop(jnp.where(ph == 0, 1, NSEG), jnp.where(ph == 0, LAG, NSEG + LAG), step_single, 0)

        @pl.when(ph == 0)
        def _():
            x_cp.wait()
            lax.fori_loop(PRE0, PRE0 + NPRE, step_both_pre, 0)
            lax.fori_loop(PRE0 + NPRE, NSEG, step_both, 0)
        return carry
    lax.fori_loop(0, 2, phase, 0)

    n_done = NSEG - 4
    cp_a = pltpu.make_async_copy(outs.at[pl.ds(0, n_done * SEG)], out_hbm.at[pl.ds(0, n_done * SEG)], osem.at[0])
    cp_a.start()
    runs = (make_stages([], [NSEG - 2, NSEG - 1], [(NSEG - 4, True), (NSEG - 3, True)]),
            make_stages([], [], [(NSEG - 2, True), (NSEG - 1, True)]))
    for which, name in ORDER_TAIL:
        runs[which](name)
    cp_b = pltpu.make_async_copy(outs.at[pl.ds(n_done * SEG, 4 * SEG)], out_hbm.at[pl.ds(n_done * SEG, 4 * SEG)],
                                 osem.at[1])
    cp_b.start()
    cp_a.wait()
    cp_b.wait()


@functools.partial(jax.jit, static_argnames=("A_seg_len",))
def pallas_interleave_layers__memory_aug_recurrent_mem_tr__mixer_s_mlp__prompt_kernel(
        A_x, A_mem0, A_Wq, A_Wk, A_Wv, A_Wo, A_seg_len, B_x, B_w1, B_w2, B_w3, B_w4):
    del B_x
    assert A_seg_len == SEG and A_x.shape == (1, S_LEN, D) and A_Wq.shape == (D, H, E)
    x = A_x.reshape(S_LEN, D)
    mem0 = A_mem0.reshape(M_MEM, D)
    wqt, wkt, wvt = (jnp.transpose(w, (1, 2, 0)).reshape(H * E, D) for w in (A_Wq, A_Wk, A_Wv))
    wo = A_Wo.reshape(H * E, D)
    any_spec = pl.BlockSpec(memory_space=pl.ANY)
    out = pl.pallas_call(
        _kernel,
        out_shape=jax.ShapeDtypeStruct((S_LEN, D), bf16),
        in_specs=[any_spec, pl.BlockSpec(memory_space=pltpu.VMEM)] + [any_spec] * 8,
        out_specs=any_spec,
        scratch_shapes=[
            pltpu.VMEM((S_LEN, D), bf16),
            pltpu.VMEM((RING, 4, PW, D), bf16),
            pltpu.VMEM((NP, 3, D // 2, PW), jnp.uint32),
            pltpu.VMEM((NP, PW // 2, D), jnp.uint32),
            pltpu.VMEM((D, D), bf16), pltpu.VMEM((D, D), bf16),
            pltpu.VMEM((D, F), bf16), pltpu.VMEM((F, D), bf16),
            pltpu.VMEM((XS_ROWS, D), f32), pltpu.VMEM((XS_ROWS, D), f32),
            pltpu.VMEM((XS_ROWS, D), f32),
            pltpu.VMEM((HB_ROWS, D), f32),
            pltpu.VMEM((2 * M_MEM, D), f32),
            pltpu.VMEM((XS_ROWS, D), bf16),
            pltpu.VMEM((3, PRE_ROWS, H * E), f32),
            pltpu.SemaphoreType.DMA((4 * RING + 3,)),
            pltpu.SemaphoreType.DMA((2,)),
        ],
        compiler_params=pltpu.CompilerParams(vmem_limit_bytes=120 * 1024 * 1024),
        name="mem_mixer",
    )(x, mem0, wqt, wkt, wvt, wo, B_w1, B_w2, B_w3, B_w4)
    return out.reshape(1, S_LEN, D)
```
